```python
import os as _os
_os.environ.setdefault("JAX_PLATFORMS", "cpu")
import jax
import jax.numpy as jnp

def _softmax(x, axis=-1):
    return jax.nn.softmax(x, axis=axis)
def _gelu(x):
    return jax.nn.gelu(x, approximate=True)
def _silu(x):
    return jax.nn.silu(x)
def _sigmoid(x):
    return jax.nn.sigmoid(x)
def _layernorm(x, axis=-1, eps=1e-5):
    m = jnp.mean(x, axis=axis, keepdims=True)
    v = jnp.var(x, axis=axis, keepdims=True)
    return (x - m) / jnp.sqrt(v + eps)
def _scatter_add(tgt, idx, src, axis=0):
    return tgt.at[idx].add(src)
def _segment_sum(src, seg, n):
    return jax.ops.segment_sum(src, seg, n)
class _Rng:
    def __init__(self, key):
        self._k = key
    def _next(self):
        self._k, sub = jax.random.split(self._k)
        return sub
    def normal(self, shape):
        return jax.random.normal(self._next(), shape, dtype=jnp.bfloat16)
    def randint(self, lo, hi, shape):
        return jax.random.randint(self._next(), shape, lo, hi, dtype=jnp.int32)
    def uniform(self, shape, lo=0.0, hi=1.0):
        return jax.random.uniform(self._next(), shape, jnp.bfloat16, lo, hi)
    def permutation(self, n):
        return jax.random.permutation(self._next(), n)


kernel_name = 'gated_mix__grouped_kv_mqa__glu_gated_reglu__prompt'

def setup_inputs():
    _rng = _Rng(jax.random.key(int.from_bytes(__import__("os").urandom(4), "little")))
    _w = (lambda a: (lambda t: t.astype(jnp.bfloat16) if jnp.issubdtype(t.dtype, jnp.floating) else t)(jnp.asarray(a)))
    def _A_setup():
        B, S, D, H = 1, 2048, 640, 32
        Dh = D // H
        return {
            "x": _w((lambda *s: _rng.normal(s) * 0.05)(B, S, D)),
            "wq": _w((lambda *s: _rng.normal(s) * 0.2)(D, H * Dh)),
            "wk": _w((lambda *s: _rng.normal(s) * 0.2)(D, Dh)),
            "wv": _w((lambda *s: _rng.normal(s) * 0.05)(D, Dh)),
            "wo": _w((lambda *s: _rng.normal(s) * 0.05)(H * Dh, D)),
        }
    _A_in = _A_setup()

    def _B_setup():
        B, S, D, F = 1, 2048, 640, 1536
        return {
            "x": _w((lambda *s: _rng.normal(s) * 0.05)(B, S, D)),
            "W_gate": _w((lambda *s: _rng.normal(s) * 0.4)(D, F) * (2.0 / D) ** 0.5),
            "W_up": _w((lambda *s: _rng.normal(s) * 0.4)(D, F) * (2.0 / D) ** 0.5),
            "W_down": _w((lambda *s: _rng.normal(s) * 0.4)(F, D) * (1.0 / F) ** 0.5),
        }
    _B_in = _B_setup()

    return {
        "A_x": _A_in["x"],
        "A_wq": _A_in["wq"],
        "A_wk": _A_in["wk"],
        "A_wv": _A_in["wv"],
        "A_wo": _A_in["wo"],
        "B_x": _B_in["x"],
        "B_W_gate": _B_in["W_gate"],
        "B_W_up": _B_in["W_up"],
        "B_W_down": _B_in["W_down"],
        "gate_w": _w((lambda *s: _rng.normal(s) * 0.05)(640) * 16.0),
    }

def reference(A_x, A_wq, A_wk, A_wv, A_wo, B_x, B_W_gate, B_W_up, B_W_down, gate_w):
    def _A_ref(x, wq, wk, wv, wo):
        B, S, D = x.shape
        H = 32
        Dh = D // H
        q = (lambda x, *d: x.transpose(*d))((x @ wq).reshape(B, S, H, Dh), 0, 2, 1, 3)
        k = x @ wk
        v = x @ wv
        scores = jnp.einsum("bhqd,bkd->bhqk", q, k) * (Dh ** -0.5)
        p = _softmax(scores, axis=-1)
        o = jnp.einsum("bhqk,bkd->bhqd", p, v)
        return (lambda x, *d: x.transpose(*d))(o, 0, 2, 1, 3).reshape(B, S, H * Dh) @ wo

    def _B_ref(x, W_gate, W_up, W_down):
        gate = jnp.einsum("bsd,df->bsf", x, W_gate)
        up = jnp.einsum("bsd,df->bsf", x, W_up)
        gate = gate * (lambda x, dt: x.astype(dt))(gate > 0, gate.dtype)
        h = gate * up
        return jnp.einsum("bsf,fd->bsd", h, W_down)

    x = A_x
    g = _sigmoid((x * gate_w).sum(-1, keepdims=True))
    a = _A_ref(x, A_wq, A_wk, A_wv, A_wo)
    b = _B_ref(x, B_W_gate, B_W_up, B_W_down)
    return g * a + (1 - g) * b
```

```python
import functools
import math

import jax
import jax.numpy as jnp
from jax import lax
import jax.experimental.pallas as pl
import jax.experimental.pallas.tpu as pltpu

S, D, H, DH, F = 2048, 640, 32, 20, 1536
TQ = 128
HS = 4
NS = H // HS
KC = 128
NC = S // KC
XC = 512
NX = S // XC
BF = jnp.bfloat16
F32 = jnp.float32
QSCALE = (DH ** -0.5) * math.log2(math.e)


def _dot(a, b):
    return lax.dot_general(a, b, (((1,), (0,)), ((), ())), preferred_element_type=F32)


def _kernel(x_hbm, wq_hbm, wk_hbm, wv_hbm, wo_hbm, wg_hbm, wu_hbm, wd_hbm, gw_hbm,
            out_ref,
            x_v, wq_v, wk_v, wv_v, wo_v, wg_v, wu_v, wd_v, gw_v,
            wkv_s, k_s, qt_s, vt_s, g_s, s_s, ot_s, sems, *, cfg):
    step = pl.program_id(0)

    def x_copy(c):
        return pltpu.make_async_copy(x_hbm.at[pl.ds(c * XC, XC), :], x_v.at[pl.ds(c * XC, XC), :], sems.at[c])

    def w_copy(i):
        src, dst = ((wq_hbm, wq_v), (wk_hbm, wk_v), (wv_hbm, wv_v), (gw_hbm, gw_v),
                    (wg_hbm, wg_v), (wu_hbm, wu_v), (wd_hbm, wd_v), (wo_hbm, wo_v))[i]
        return pltpu.make_async_copy(src, dst, sems.at[NX + i])

    @pl.when(step == 0)
    def _prologue():
        x_copy(0).start()
        s_s[0, pl.ds(pl.multiple_of(step * 8, 8), 8), :] = jnp.zeros((8, HS * TQ), F32)
        for i in range(4):
            w_copy(i).start()
        for i in (1, 2, 3):
            w_copy(i).wait()
        for c in range(1, NX):
            x_copy(c).start()
        wk = wk_v[...].astype(F32)
        wv = wv_v[...].astype(F32)
        gw = jnp.broadcast_to(gw_v[...].astype(F32).reshape(1, D), (4, D))
        pad = jnp.zeros((128 - 5 * DH - 4, D), F32)
        wkv_s[...] = jnp.concatenate([wk, wk, wk, wk, wv, gw, pad], axis=0).T.astype(BF)
        w_copy(0).wait()

        for c in range(NX):
            x_copy(c).wait()
            if c == 1:
                for i in range(4, 8):
                    w_copy(i).start()
            xc = x_v[pl.ds(c * XC, XC), :]
            kv = _dot(xc, wkv_s[...])
            q = _dot(xc, wq_v[...]) * QSCALE
            lane = lax.broadcasted_iota(jnp.int32, kv.shape, 1)
            k_s[pl.ds(c * XC // 2, XC // 2), :] = pltpu.bitcast(
                jnp.where(lane < HS * DH, kv, 0.0).astype(BF), jnp.uint32)
            g_s[pl.ds(c * XC, XC), :] = jax.nn.sigmoid(jnp.broadcast_to(kv[:, 5 * DH:5 * DH + 1], kv.shape))
            kvt = kv.T
            row = lax.broadcasted_iota(jnp.int32, (24, XC), 0)
            v = kvt[80:104].astype(BF).astype(F32)
            vt_s[0, :, pl.ds(c * XC, XC)] = jnp.where(row < DH, v, 1.0)
            qt = pltpu.bitcast(q.T.astype(BF), jnp.uint32)
            for b in range(XC // TQ):
                qt_s[c * (XC // TQ) + b] = qt[:, b * TQ:(b + 1) * TQ]
        for i in range(4, 8):
            w_copy(i).wait()

    row0 = pl.multiple_of(step * TQ, TQ)
    zeros8 = jnp.zeros((8, TQ), jnp.uint32)
    urow = lax.broadcasted_iota(jnp.int32, (8, TQ), 0)

    def q_weights(s):
        cols = []
        for j in range(HS):
            tiles = []
            for r in range(8):
                lo, hi = 10 * j - 8 * r, 10 * j + 10 - 8 * r
                if hi <= 0 or lo >= 8:
                    tiles.append(zeros8)
                else:
                    t = qt_s[step, pl.ds(40 * s + 8 * r, 8), :]
                    keep = (urow >= lo) if lo > 0 else (urow < hi)
                    tiles.append(jnp.where(keep, t, zeros8))
            cols.append(jnp.concatenate(tiles, axis=0))
        return pltpu.bitcast(jnp.concatenate(cols, axis=1), BF)

    qw, mx, acc = {}, {}, {}

    def qk(s, c):
        if c == 0:
            qw[s] = q_weights(s)
        kk = pltpu.bitcast(k_s[pl.ds(c * KC // 2, KC // 2), :], BF)
        sc = _dot(kk, qw[s])
        s_s[s % 2, pl.ds(c * KC, KC), :] = sc
        m = sc[0:8]
        for i in range(1, KC // 8):
            m = jnp.maximum(m, sc[8 * i:8 * i + 8])
        mx[s] = m if c == 0 else jnp.maximum(mx[s], m)
        if c == NC - 1:
            mx[s] = jnp.broadcast_to(jnp.max(mx[s], axis=0, keepdims=True), (8, HS * TQ))

    def pv(s, c):
        sc = s_s[s % 2, pl.ds(c * KC, KC), :]
        p = jnp.exp2(sc - jnp.concatenate([mx[s]] * (KC // 8), axis=0)).astype(BF)
        r = _dot(vt_s[0, :, pl.ds(c * KC, KC)], p)
        acc[s] = r if c == 0 else acc[s] + r

    def norm(s):
        a = acc.pop(s)
        o = a[0:24] * (1.0 / a[DH:DH + 1])
        for j in range(HS):
            h = s * HS + j
            ot_s[pl.ds(h * DH, DH), :] = o[0:DH, j * TQ:(j + 1) * TQ]

    xq = x_v[pl.ds(row0, TQ), :]
    FC = cfg.get("FC", 512)
    hs = {}
    ffn = {}

    def ffn_up(f):
        gate = _dot(xq, wg_v[:, pl.ds(f * FC, FC)])
        up = _dot(xq, wu_v[:, pl.ds(f * FC, FC)])
        hs[f] = (jnp.where(gate > 0, gate, 0.0) * up).astype(BF)

    def ffn_down(f):
        r = _dot(hs.pop(f), wd_v[pl.ds(f * FC, FC), :])
        ffn["b"] = r if f == 0 else ffn["b"] + r

    for s in range(NS + 1):
        for c in range(NC):
            if s < NS:
                qk(s, c)
            if s > 0:
                pv(s - 1, c)
            if s > 1 and c == cfg.get("ND", 4):
                norm(s - 2)
            if s == NS:
                if c == 0:
                    ffn_up(0)
                if c == 8:
                    ffn_up(1)
    ffn_up(2)
    norm(NS - 1)
    for f in range(F // FC):
        ffn_down(f)
    o = ot_s[...].T.astype(BF)
    a = _dot(o, wo_v[...])
    g = g_s[pl.ds(row0, TQ), :]
    g = jnp.concatenate([g] * (D // 128), axis=1)
    out_ref[...] = (g * a + (1.0 - g) * ffn["b"]).astype(out_ref.dtype)


def build(**cfg):
    def fn(A_x, A_wq, A_wk, A_wv, A_wo, B_x, B_W_gate, B_W_up, B_W_down, gate_w):
        del B_x
        any_spec = pl.BlockSpec(memory_space=pl.ANY)
        out = pl.pallas_call(
            functools.partial(_kernel, cfg=cfg),
            grid=(S // TQ,),
            in_specs=[any_spec] * 9,
            out_specs=pl.BlockSpec((TQ, D), lambda i: (i, 0)),
            out_shape=jax.ShapeDtypeStruct((S, D), A_x.dtype),
            scratch_shapes=[
                pltpu.VMEM((S, D), BF), pltpu.VMEM((D, D), BF), pltpu.VMEM((DH, D), BF), pltpu.VMEM((DH, D), BF),
                pltpu.VMEM((D, D), BF), pltpu.VMEM((D, F), BF), pltpu.VMEM((D, F), BF), pltpu.VMEM((F, D), BF),
                pltpu.VMEM((D,), BF),
                pltpu.VMEM((D, 128), BF),
                pltpu.VMEM((S // 2, 128), jnp.uint32),
                pltpu.VMEM((S // TQ, D // 2, TQ), jnp.uint32),
                pltpu.VMEM((1, 24, S), F32),
                pltpu.VMEM((S, 128), F32),
                pltpu.VMEM((2, S, HS * TQ), F32),
                pltpu.VMEM((D, TQ), F32),
                pltpu.SemaphoreType.DMA((NX + 8,)),
            ],
            compiler_params=pltpu.CompilerParams(
                dimension_semantics=("arbitrary",), vmem_limit_bytes=100 * 2**20, flags=cfg.get("flags")),
        )(A_x.reshape(S, D), A_wq, A_wk.T, A_wv.T, A_wo, B_W_gate, B_W_up, B_W_down, gate_w)
        return out.reshape(1, S, D)
    return jax.jit(fn)


pallas_gated_mix__grouped_kv_mqa__glu_gated_reglu__prompt_kernel = build()
```

```python
import functools
import math

import jax
import jax.numpy as jnp
from jax import lax
import jax.experimental.pallas as pl
import jax.experimental.pallas.tpu as pltpu

S, D, H, DH, F = 2048, 640, 32, 20, 1536
TQ = 128
NQ = S // TQ
HS = 4
NS = H // HS
NT = S // 128
XC = 512
NX = S // XC
RING = 4
BF = jnp.bfloat16
F32 = jnp.float32
U32 = jnp.uint32
QSCALE = (DH ** -0.5) * math.log2(math.e)
L_MIN, L_MAX = 2.0 ** -20, 2.0 ** 90

A_K = 0
A_X = A_K + S // 2
A_H = A_X + NQ * 5 * 64
A_P = A_H + 12 * 64
A_ROWS = A_P + NS * NT * 2 * HS * 8
QO_O = HS * DH * 8


def _dot(a, b):
    return lax.dot_general(a, b, (((1,), (0,)), ((), ())), preferred_element_type=F32)


def _kernel(x_hbm, wq_hbm, wk_hbm, wv_hbm, wo_hbm, wg_hbm, wu_hbm, wd_hbm, gw_hbm,
            out_ref,
            x_v, wq_v, wo_v, wg_v, wu_v, wd_v,
            wkv_s, a_s, kb_s, qt_s, qf_s, vt_s, g_s, ot_s, b_s, tmp_s, tmp2_s, sems, *rest, cfg):
    step = pl.program_id(0)
    ring, qo_s = rest[:RING], rest[RING:RING + NS]
    wk_v, wv_v, gw_v = rest[RING + NS:]
    lag = cfg.get("lag", 3)
    ns = cfg.get("ns", NS)
    n_blocks = cfg.get("blocks", 128)
    n_tail = cfg.get("tail", 5)
    uw = cfg.get("uw", 2)

    def x_copy(c):
        return pltpu.make_async_copy(x_hbm.at[pl.ds(c * XC, XC), :], x_v.at[pl.ds(c * XC, XC), :], sems.at[c])

    def w_copy(i):
        src, dst = ((wq_hbm, wq_v), (wk_hbm, wk_v), (wv_hbm, wv_v), (gw_hbm, gw_v),
                    (wg_hbm, wg_v), (wu_hbm, wu_v), (wd_hbm, wd_v), (wo_hbm, wo_v))[i]
        return pltpu.make_async_copy(src, dst, sems.at[NX + i])

    def spread_q(blk_idx, r):
        blk = qf_s[blk_idx, pl.ds(8 * r, 8), :]
        for u in range(8):
            qo_s[r // 10][pl.ds(64 * (r % 10) + 8 * u, 8), :] = pltpu.bitcast(
                jnp.broadcast_to(blk[u:u + 1], (8, TQ)), U32)

    @pl.when(step == 0)
    def _prologue():
        x_copy(0).start()
        for i in range(4):
            w_copy(i).start()
        for i in (1, 2, 3):
            w_copy(i).wait()
        for c in range(1, NX):
            x_copy(c).start()
        wk = wk_v[...].astype(F32)
        wv = wv_v[...].astype(F32)
        gw = jnp.broadcast_to(gw_v[...].astype(F32).reshape(1, D), (8, D))
        wkv_s[...] = jnp.concatenate([wk, wk, wk, wk, wv, gw, wv], axis=0).T.astype(BF)
        w_copy(0).wait()

        def chunk(c, carry):
            x_copy(c).wait()

            @pl.when(c == 1)
            def _():
                for i in range(4, 8):
                    w_copy(i).start()

            r0 = pl.multiple_of(c * XC, XC)
            xc = x_v[pl.ds(r0, XC), :]
            xu = pltpu.bitcast(xc, U32)
            kv = _dot(xc, wkv_s[...])
            q = _dot(xc, wq_v[...]) * QSCALE
            lane = lax.broadcasted_iota(jnp.int32, kv.shape, 1)
            kz = jnp.where(lane < HS * DH, kv, 0.0).astype(BF)
            a_s[pl.ds(pl.multiple_of(A_K + c * (XC // 2), 8), XC // 2), :] = pltpu.bitcast(kz, U32)
            g_s[pl.ds(r0, XC), :] = jax.nn.sigmoid(jnp.broadcast_to(kv[:, 5 * DH:5 * DH + 1], kv.shape))
            v1 = jnp.where((lane >= 5 * DH) & (lane < 5 * DH + 8), 1.0, kv.astype(BF).astype(F32))
            qt = q.T.astype(BF)
            qu = pltpu.bitcast(qt, U32)
            qf = qt.astype(F32)
            for b in range(XC // 128):
                t = c * (XC // 128) + b
                vt_s[t] = v1[b * 128:(b + 1) * 128].T[80:128]
                kk = kz[b * 128 + 96:(b + 1) * 128].astype(F32)
                for d in range(DH):
                    kd = jnp.broadcast_to(kk[:, d:d + 1], (32, 128))
                    kb_s[pl.ds(pl.multiple_of(t * 2 * DH * 16, 32) + (DH + d) * 16, 16), :] = kd[0:16]
                    kb_s[pl.ds(pl.multiple_of(t * 2 * DH * 16, 32) + d * 16, 16), :] = kd[16:32]
                for k in range(5):
                    a_s[pl.ds(pl.multiple_of(A_X + (t * 5 + k) * 64, 8), 64), :] = (
                        xu[b * 64:(b + 1) * 64, k * 128:(k + 1) * 128])
                qt_s[t] = qu[:, b * TQ:(b + 1) * TQ]
                qf_s[t] = qf[:, b * TQ:(b + 1) * TQ]
            return carry

        lax.fori_loop(0, NX, chunk, 0)
        for r in range(D // 8):
            spread_q(0, r)
        for i in range(4, 8):
            w_copy(i).wait()

    row0 = pl.multiple_of(step * TQ, TQ)
    zeros8 = jnp.zeros((8, TQ), U32)
    urow = lax.broadcasted_iota(jnp.int32, (8, TQ), 0)
    nz = [0]

    def fresh_zero():
        nz[0] += 1
        return pl.multiple_of(((step + nz[0]) >> 16) * 32, 32)

    zero = fresh_zero()

    def q_weights(s):
        base = 40 * s if isinstance(s, int) else pl.multiple_of(40 * s, 8)
        cols = []
        for j in range(HS):
            tiles = []
            for r in range(8):
                lo, hi = 10 * j - 8 * r, 10 * j + 10 - 8 * r
                if hi <= 0 or lo >= 8:
                    tiles.append(zeros8)
                else:
                    t = qt_s[step, pl.ds(base + 8 * r, 8), :]
                    keep = (urow >= lo) if lo > 0 else (urow < hi)
                    tiles.append(jnp.where(keep, t, zeros8))
            cols.append(jnp.concatenate(tiles, axis=0))
        return pltpu.bitcast(jnp.concatenate(cols, axis=1), BF)

    qw, acc, chk, dense = {}, {}, {}, {}
    items = [(s, t) for s in range(ns) for t in range(NT)]
    n = len(items)
    nb = [(i + 1) * n_blocks // n - i * n_blocks // n for i in range(n)]

    def p_row(i, b, j):
        return A_P + ((i * 2 + b) * HS + j) * 8

    views = {}

    def vpu_unit(i, b, j0):
        s, t = items[i]
        z = fresh_zero()
        qv = qo_s[s].at[pl.ds(z, QO_O)]
        kv_ = kb_s.at[pl.ds(z + (t * 2 + b) * DH * 16, DH * 16)]
        a = None
        for d in range(DH):
            q = jnp.concatenate(
                [pltpu.bitcast(qv[pl.ds((j * DH + d) * 8, 8), :], F32) for j in range(j0, j0 + uw)], axis=1)
            term = jnp.concatenate([kv_[pl.ds(16 * d, 16), :]] * uw, axis=1) * jnp.concatenate([q, q], axis=0)
            a = term if a is None else a + term
        e = jnp.exp2(a)
        if uw == 1:
            e = jnp.concatenate([e, e], axis=1)
        tmp_s[...] = pltpu.bitcast(e.astype(BF), U32)
        for j in range(uw):
            a_s[pl.ds(p_row(i, b, j0 + j), 8), :] = tmp_s[:, pl.ds(j * TQ, TQ)]

    units = [(i, b, j0) for i in range(n) for b in range(nb[i]) for j0 in range(0, HS, uw)]
    head = 45 - n_tail
    last = n - cfg.get("endgap", 0)
    w_d, w_q, w_p = cfg.get("wts", (50, 52, 84))
    total = head * 8 * w_d + sum((8 - nb[i]) * w_q + (w_p if i >= lag else 0) for i in range(last))
    pace = {"credit": cfg.get("c0", 0.0) * total / max(len(units), 1), "done": 0}

    def run_units(upto):
        while pace["done"] < min(upto, len(units)):
            vpu_unit(*units[pace["done"]])
            pace["done"] += 1

    def paced_lhs(load, slots, weight):
        rows = []
        for r in range(slots):
            pace["credit"] += weight
            run_units(int(pace["credit"] * len(units) / total))
            rows.append(load(8 * r))
        return pltpu.bitcast(jnp.concatenate(rows, axis=0), BF)

    def qk(i, s, t):
        if t == 0:
            qw[s] = q_weights(s)
        slots = 8 - nb[i]
        av = a_s.at[pl.ds(zero + A_K + t * 64, 64)]
        kk = paced_lhs(lambda r: av[pl.ds(r, 8), :], slots, w_q)
        p = jnp.exp2(_dot(kk, qw[s])).astype(BF)
        ring[i % RING][pl.ds(0, slots * 8), :] = pltpu.bitcast(p, U32)

    def pv(i, s, t):
        need = sum(1 for u in units if u[0] <= i)
        if pace["done"] < need:
            print("late", i, need - pace["done"])
            run_units(need)
        pace["credit"] += w_p
        pm = ring[i % RING][pl.ds(zero, (8 - nb[i]) * 8), :]
        for j in range(HS):
            parts = [pm[:, j * TQ:(j + 1) * TQ]]
            parts += [a_s[pl.ds(p_row(i, b, j), 8), :] for b in reversed(range(nb[i]))]
            w = pltpu.bitcast(jnp.concatenate(parts, axis=0), BF)
            r = _dot(vt_s[t, pl.ds(24 * (j % 2), 24), :], w)
            acc[s, j] = r if t == 0 else acc[s, j] + r

    def norm(s):
        for j in range(0, HS, 2):
            ev, od = acc.pop((s, j)), acc.pop((s, j + 1))
            ll = jnp.where(urow < 4, od[0:8], ev[16:24])
            chk["lo"] = ll if "lo" not in chk else jnp.minimum(chk["lo"], ll)
            chk["hi"] = ll if "hi" not in chk else jnp.maximum(chk["hi"], ll)
            inv = 1.0 / ll
            ev = ev * jnp.broadcast_to(inv[4:5], (24, TQ))
            od = od * jnp.broadcast_to(inv[0:1], (24, TQ))
            o = jnp.concatenate([ev[0:16], jnp.where(urow < 4, ev[16:24], od[0:8]), od[8:24]], axis=0)
            ot_s[pl.ds((s * HS + j) * DH, 2 * DH), :] = o
            for r in range(5):
                z = o[8 * r:8 * r + 8] * 0.0
                chk["fin"] = z if "fin" not in chk else chk["fin"] + z

    xv = a_s.at[pl.ds(pl.multiple_of(A_X + step * 320, 8), 320)]
    hv = a_s.at[pl.ds(zero + A_H, 768)]

    def put_h(f):
        tmp2_s[:, pl.ds(0, 512)] = dense.pop(("h", f))
        for k in range(4):
            a_s[pl.ds(A_H + (4 * f + k) * 64, 64), :] = tmp2_s[:, pl.ds(k * 128, 128)]

    def ffn_gu(f, which, k, weight):
        w = (wg_v, wu_v)[which]
        lhs = paced_lhs(lambda r: xv[pl.ds(k * 64 + r, 8), :], 8, weight)
        r = _dot(lhs, w[pl.ds(k * 128, 128), pl.ds(f * 512, 512)])
        dense[which] = r if k == 0 else r + dense[which]
        if which == 1 and k == 4:
            gate, up = dense.pop(0), dense.pop(1)
            dense["h", f] = pltpu.bitcast((jnp.where(gate > 0, gate, 0.0) * up).astype(BF), U32)
        if which == 0 and k == 1 and f > 0:
            put_h(f - 1)

    def ffn_dn(f, n_, weight):
        if f == 0 and n_ == 2:
            put_h(2)
        lhs = paced_lhs(lambda r: jnp.concatenate(
            [hv[pl.ds((4 * f + k) * 64 + r, 8), :] for k in range(4)], axis=1), 8, weight)
        r = _dot(lhs, wd_v[pl.ds(f * 512, 512), pl.ds(n_ * 128, 128)])
        cs = pl.ds(n_ * 128, 128)
        b_s[:, cs] = r if f == 0 else b_s[:, cs] + r

    jobs = [functools.partial(ffn_gu, f, w, k) for f in range(3) for w in range(2) for k in range(5)]
    jobs += [functools.partial(ffn_dn, f, n_) for f in range(3) for n_ in range(5)]

    for job in jobs[:head]:
        job(w_d)
    issued = head
    for i in range(n + lag):
        if i < n:
            qk(i, *items[i])
        else:
            jobs[issued](w_d)
            issued += 1
        if i >= lag:
            s, t = items[i - lag]
            pv(i - lag, s, t)
            if t == 2 and s > 0:
                norm(s - 1)
    for job in jobs[issued:]:
        job(w_d)
    norm(ns - 1)

    def combine(a, cs):
        g = g_s[pl.ds(row0, TQ), :]
        g = jnp.concatenate([g] * (a.shape[1] // 128), axis=1)
        out_ref[:, cs] = (g * a + (1.0 - g) * b_s[:, cs]).astype(out_ref.dtype)

    tmp2_s[...] = pltpu.bitcast(ot_s[...].T.astype(BF), U32)
    op = tmp2_s[...]
    for k in range(5):
        for r in range(8):
            qo_s[r][pl.ds(QO_O + 8 * k, 8), :] = op[8 * r:8 * r + 8, k * 128:(k + 1) * 128]
    nxt = jnp.minimum(step + 1, NQ - 1)
    lhs = []
    a = None
    for k in range(5):
        rows = []
        for r in range(8):
            spread_q(nxt, 10 * r + 2 * k)
            spread_q(nxt, 10 * r + 2 * k + 1)
            rows.append(qo_s[r][pl.ds(zero + QO_O + 8 * k, 8), :])
        lhs.append(pltpu.bitcast(jnp.concatenate(rows, axis=0), BF))
        r = _dot(lhs[k], wo_v[pl.ds(k * 128, 128), pl.ds(0, 512)])
        a = r if k == 0 else r + a
    combine(a, pl.ds(0, 512))
    a = _dot(jnp.concatenate(lhs[:4], axis=1), wo_v[pl.ds(0, 512), pl.ds(512, 128)])
    w4 = wo_v[pl.ds(512, 128), pl.ds(512, 128)]
    a = a + jnp.concatenate([_dot(lhs[4][32 * r:32 * r + 32], w4) for r in range(4)], axis=0)
    combine(a, pl.ds(512, 128))

    safe = (chk["lo"] >= L_MIN) & (chk["hi"] <= L_MAX) & (chk["fin"] == 0.0)
    unsafe = jnp.max(jnp.where(safe, 0.0, 1.0))

    @pl.when(unsafe > 0.0)
    def _exact_max():
        def slab(s, carry):
            w = q_weights(s)

            def scores(t):
                return _dot(pltpu.bitcast(a_s[pl.ds(pl.multiple_of(A_K + t * 64, 64), 64), :], BF), w)

            m = lax.fori_loop(0, NT, lambda t, m: jnp.maximum(m, jnp.max(scores(t), axis=0, keepdims=True)),
                              jnp.full((1, HS * TQ), -jnp.inf, F32))
            a = lax.fori_loop(
                0, NT, lambda t, a: a + _dot(vt_s[t, pl.ds(0, 24), :], jnp.exp2(scores(t) - m).astype(BF)),
                jnp.zeros((24, HS * TQ), F32))
            o = a * (1.0 / a[DH:DH + 1])
            o = jnp.concatenate([o[:DH, j * TQ:(j + 1) * TQ] for j in range(HS)], axis=0)
            ot_s[pl.ds(pl.multiple_of(s * HS * DH, 8), HS * DH), :] = o
            return carry

        lax.fori_loop(0, NS, slab, 0)
        combine(_dot(ot_s[...].T.astype(BF), wo_v[...]), pl.ds(0, D))


def build(**cfg):
    def fn(A_x, A_wq, A_wk, A_wv, A_wo, B_x, B_W_gate, B_W_up, B_W_down, gate_w):
        del B_x
        any_spec = pl.BlockSpec(memory_space=pl.ANY)
        out = pl.pallas_call(
            functools.partial(_kernel, cfg=cfg),
            grid=(NQ,),
            in_specs=[any_spec] * 9,
            out_specs=pl.BlockSpec((TQ, D), lambda i: (i, 0)),
            out_shape=jax.ShapeDtypeStruct((S, D), A_x.dtype),
            scratch_shapes=[
                pltpu.VMEM((S, D), BF), pltpu.VMEM((D, D), BF),
                pltpu.VMEM((D, D), BF), pltpu.VMEM((D, F), BF), pltpu.VMEM((D, F), BF), pltpu.VMEM((F, D), BF),
                pltpu.VMEM((D, 128), BF),
                pltpu.VMEM((A_ROWS, 128), U32),
                pltpu.VMEM((NT * 2 * DH * 16, 128), F32),
                pltpu.VMEM((NQ, D // 2, TQ), U32),
                pltpu.VMEM((NQ, D, TQ), F32),
                pltpu.VMEM((NT, 48, 128), F32),
                pltpu.VMEM((S, 128), F32),
                pltpu.VMEM((D, TQ), F32),
                pltpu.VMEM((TQ, D), F32),
                pltpu.VMEM((8, max(2, cfg.get("uw", 2)) * TQ), U32),
                pltpu.VMEM((TQ // 2, D), U32),
                pltpu.SemaphoreType.DMA((NX + 8,)),
            ] + [pltpu.VMEM((64, HS * TQ), U32)] * RING + [pltpu.VMEM((QO_O + 64, TQ), U32)] * NS + [
                pltpu.VMEM((DH, D), BF), pltpu.VMEM((DH, D), BF), pltpu.VMEM((D,), BF)],
            compiler_params=pltpu.CompilerParams(
                dimension_semantics=("arbitrary",), vmem_limit_bytes=100 * 2**20, flags=cfg.get("flags")),
        )(A_x.reshape(S, D), A_wq, A_wk.T, A_wv.T, A_wo, B_W_gate, B_W_up, B_W_down, gate_w)
        return out.reshape(1, S, D)
    return jax.jit(fn)


pallas_gated_mix__grouped_kv_mqa__glu_gated_reglu__prompt_kernel = build(blocks=192,wts=(40,52,84))
```

```python
import functools
import math

import jax
import jax.experimental.pallas as pl
import jax.experimental.pallas.tpu as pltpu
import jax.numpy as jnp
from jax import lax

S, D, H, DH, F = 2048, 640, 32, 20, 1536
TQ = 128
NQ = S // TQ
HS = 4
NS = H // HS
NT = S // 128
HD = DH // 2
X_FIRST = 512
BF16, F32, U32 = jnp.bfloat16, jnp.float32, jnp.uint32
Q_SCALE = DH ** -0.5 * math.log2(math.e)

SUM_MIN, SUM_MAX, V_MAX = 2.0 ** -20, 2.0 ** 90, 2.0 ** 30

VPU_TILES = 111
AHEAD = 4
LAG = 3
RING = LAG + 1
DOWN_AT = 2
O_INSIDE = 2
O_FIRST = 0
TAIL_SLOTS = 3
W_DENSE, W_QK, W_PV = 52, 52, 84
C_SPREAD = 24

L_K = 0
L_X = L_K + S // 2
L_ZERO = L_X + NQ * 512
L_SINK = L_ZERO + 32
L_P = L_SINK + 32
L_ROWS = L_P + NS * NT * 64
TERM_ROWS = 7 * HD * 16


def _dot(a, b):
    return lax.dot_general(a, b, (((1,), (0,)), ((), ())), preferred_element_type=F32)


def _dot_nt(a, b):
    return lax.dot_general(a, b, (((1,), (1,)), ((), ())), preferred_element_type=F32)


def _pack(val):
    return pltpu.bitcast(val.astype(BF16), U32)


def _unpack(words):
    return pltpu.bitcast(words, BF16)


def _strassen_lhs(a11, a12, a21, a22):
    return a11 + a22, a21 + a22, a11, a22, a11 + a12, a21 - a11, a12 - a22


def _strassen_rhs(b11, b12, b21, b22):
    return b11 + b22, b11, b12 - b22, b21 - b11, b22, b11 + b12, b21 + b22


def _winograd_lhs(a11, a12, a21, a22):
    s1 = a21 + a22
    s2 = s1 - a11
    return a11, a12, a12 - s2, a22, s1, s2, a11 - a21


def _winograd_rhs(b11, b12, b21, b22):
    t1 = b12 - b11
    t2 = b22 - t1
    return b11, b21, b22, b21 - t2, t1, t2, b22 - b12


def _kernel(x_hbm, wq_hbm, wk_hbm, wv_hbm, gw_hbm, wg_hbm, wu_hbm, wd_hbm, wo_hbm, out_ref,
            x_v, wq_v, wg_v, wu_v, wd_v, wo_v,
            wqt_s, qpart_s, lhs_s, lhs2_s, kb_s, qt_s, qf_s, vt_s, g_s,
            wgu_s, wgu_rest_s, wd_s, wd_rest_s, wo_s,
            ot_s, o_s, a_s, gu_s, vbig_s, ring_s, qb_s, b_s, h_s, park_s, stage_s,
            wkv_v, gw_v, sems):
    step = pl.program_id(0)
    tiles = [(s, t) for s in range(NS) for t in range(NT)]
    n = len(tiles)
    on_vpu = [(n - i) * VPU_TILES // n > (n - i - 1) * VPU_TILES // n for i in range(n)]
    slots = [6 if v else 8 for v in on_vpu]
    n_zero = [0]

    def opaque_zero():
        n_zero[0] += 1
        return pl.multiple_of(((step + n_zero[0]) >> 16) * 32, 32)

    def staged_pack(stage, val):
        stage[...] = _pack(val)
        return stage[...]

    def spread_q(block, s, d):
        for c in range(2):
            b11, b21, b12, b22 = [
                jnp.broadcast_to(qf_s[block, pl.ds(DH * (HS * s + c + 2 * u) + HD * v + d, 1), :], (8, TQ))
                for u in range(2) for v in range(2)]
            for m, val in enumerate(_winograd_rhs(b11, b12, b21, b22)):
                qb_s[s][pl.ds((m * HD + d) * 16 + 8 * c, 8), :] = val

    def vpu_scores(i, stage):
        s, t = tiles[i]
        live = {}

        def product(m, acc):
            zero = opaque_zero()
            rows = pl.ds(m * HD * 16, HD * 16)
            q = qb_s[s].at[pl.ds(zero, TERM_ROWS)][rows, :].reshape(HD, 16, TQ)
            k = kb_s.at[pl.ds(zero + t * TERM_ROWS, TERM_ROWS)][rows, :].reshape(HD, 16, TQ)
            q = jnp.concatenate([q[:, :8], q[:, 8:]], axis=2)
            q = jnp.concatenate([q, q], axis=1)
            k = jnp.concatenate([k, k], axis=2)
            for d in range(HD):
                acc = k[d] * q[d] if acc is None else acc + k[d] * q[d]
            return acc

        def emit(scores, u, j):
            p = staged_pack(stage, jnp.exp2(scores))
            for c in range(2):
                lhs_s[pl.ds(L_P + 64 * i + 32 * u + 8 * (j + c), 8), :] = p[:, c * TQ:(c + 1) * TQ]

        def c11():
            live["m1"] = product(0, None)
            emit(product(1, live["m1"]), 0, 0)

        def c12():
            live["u2"] = product(5, live.pop("m1"))
            live["m5"] = product(4, None)
            emit(product(2, live["u2"] + live["m5"]), 0, 2)

        def c22():
            live["u3"] = product(6, live.pop("u2"))
            emit(live["u3"] + live.pop("m5"), 1, 2)

        def c21():
            emit(product(3, live.pop("u3")), 1, 0)

        return [(162, c11), (246, c12), (90, c22), (86, c21)]

    @pl.when(step == 0)
    def _load_and_project():
        first, rest = pl.ds(0, X_FIRST), pl.ds(X_FIRST, S - X_FIRST)
        wq, wk, wv, gw, x0, x1, wg, wu, wd, wo = [
            pltpu.make_async_copy(src, dst, sems.at[i]) for i, (src, dst) in enumerate((
                (wq_hbm, wq_v), (wk_hbm, wkv_v.at[0]), (wv_hbm, wkv_v.at[1]), (gw_hbm, gw_v),
                (x_hbm.at[first, :], x_v.at[first, :]), (x_hbm.at[rest, :], x_v.at[rest, :]),
                (wg_hbm, wg_v), (wu_hbm, wu_v), (wd_hbm, wd_v), (wo_hbm, wo_v)))]
        for copy in (wq, wk, wv, gw, x0, x1):
            copy.start()
        lhs_s[pl.ds(L_ZERO, 8), :] = jnp.zeros((8, 128), U32)
        for copy in (wq, wk, wv, gw):
            copy.wait()
        wkv = jnp.concatenate(
            [wkv_v[0].astype(F32), jnp.broadcast_to(gw_v[...].astype(F32).reshape(1, D), (8, D)),
             wkv_v[1].astype(F32)], axis=0).astype(BF16)
        wqt_s[pl.ds(0, D // 2), :] = pltpu.bitcast(wq_v[...].T, U32)
        lane = lax.broadcasted_iota(jnp.int32, (64, 128), 1)
        row = lax.broadcasted_iota(jnp.int32, (24, 128), 0)
        v_big = [jnp.zeros((8, 128), F32)]

        def project_kv(t0):
            kv = _dot_nt(wkv, x_v[pl.ds(128 * t0, 512), :])
            for t in range(t0, t0 + 4):
                kvt = kv[:, 128 * (t - t0):128 * (t - t0 + 1)]
                v_odd = jnp.where(row < 4, 1.0, kvt[24:48])
                vt_s[t, pl.ds(24, 24), :] = v_odd
                vt_s[t, pl.ds(0, 24), :] = jnp.concatenate([v_odd[4:24], jnp.ones((4, 128), F32)], axis=0)
                for r in range(3):
                    v_big[0] = jnp.where(jnp.abs(v_odd[8 * r:8 * r + 8]) <= V_MAX, v_big[0], 1.0)
                k = jnp.concatenate([kvt[0:DH]] * HS + [jnp.zeros((120 - HS * DH, 128), F32),
                                                        jax.nn.sigmoid(kvt[16:24])], axis=0).T
                g_s[pl.ds(128 * t, 128), :] = jnp.broadcast_to(k[:, 124:125], (128, 128))
                words = jnp.where(lane < HS * DH, _pack(k), jnp.zeros((64, 128), U32))
                lhs_s[pl.ds(L_K + 64 * t, 64), :] = words
                lhs2_s[pl.ds(L_K + 64 * t, 64), :] = words
                for d in range(HD):
                    lo = jnp.broadcast_to(k[96:, d:d + 1], (32, 128))
                    hi = jnp.broadcast_to(k[96:, HD + d:HD + d + 1], (32, 128))
                    for m, val in enumerate(_winograd_lhs(lo[:16], hi[:16], lo[16:], hi[16:])):
                        kb_s[pl.ds(t * TERM_ROWS + (m * HD + d) * 16, 16), :] = val

        def x_terms(t0, t1):
            for t in range(t0, t1):
                for r in range(0, 64, 16):
                    blocks = [x_v[pl.ds(128 * t + 64 * u + r, 16), pl.ds(256 * v, 256)].astype(F32)
                              for u in range(2) for v in range(2)]
                    for m, val in enumerate(_strassen_lhs(*blocks)):
                        val = staged_pack(stage_s[1], val)
                        for u, dst in enumerate((lhs_s, lhs2_s)):
                            dst[pl.ds(L_X + 512 * t + 64 * m + 32 * u + r // 2, 8), :] = (
                                val[:, 128 * u:128 * (u + 1)])
                    lhs_s[pl.ds(L_X + 512 * t + 448 + r, 16), :] = pltpu.bitcast(
                        x_v[pl.ds(128 * t + 2 * r, 32), pl.ds(512, 128)], U32)

        def gate_up_terms(which, c, r):
            w = (wg_v, wu_v)[which]
            blocks = [w[pl.ds(256 * u + r, 16), pl.ds(128 * (c + 6 * v), 256)].astype(F32)
                      for u in range(2) for v in range(2)]
            for m, val in enumerate(_strassen_rhs(*blocks)):
                val = staged_pack(stage_s[1], val)
                for u in range(2):
                    wgu_s[c + u, m, pl.ds(r // 2, 8), pl.ds(128 * which, 128)] = val[:, 128 * u:128 * (u + 1)]
            if r < 128:
                for v in range(2):
                    val = staged_pack(stage_s[1], w[pl.ds(512 + r, 16), pl.ds(128 * (c + 6 * v), 256)].astype(F32))
                    for u in range(2):
                        wgu_rest_s[c + u, pl.ds(r // 2, 8), pl.ds(256 * v + 128 * which, 128)] = (
                            val[:, 128 * u:128 * (u + 1)])
            wqt_s[pl.ds(D // 2, 8), pl.ds(0, 128)] = wgu_s[c, 0, pl.ds(opaque_zero(), 8), pl.ds(0, 128)]

        def project_q(t0, work=()):
            def lhs(c0, nc, part):
                per = len(work) / (4 * D // 16)
                view = wqt_s.at[pl.ds(opaque_zero(), D // 2)]
                rows = []
                for r in range(D // 16):
                    if part is not None:
                        at = part * D // 16 + r
                        for item in work[int(at * per):int((at + 1) * per)]:
                            item()
                    rows.append(view[pl.ds(8 * r, 8), pl.ds(c0, nc)])
                return _unpack(jnp.concatenate(rows, axis=0))

            q_rest = _dot_nt(lhs(512, 128, None), x_v[pl.ds(128 * t0, 512), pl.ds(512, 128)])
            for u in range(4):
                qpart_s[u] = q_rest[:, 128 * u:128 * (u + 1)]
            for u in range(4):
                q = qpart_s[u, pl.ds(opaque_zero(), D), :] + _dot_nt(
                    lhs(0, 512, u), x_v[pl.ds(128 * (t0 + u), 128), pl.ds(0, 512)])
                q = q * Q_SCALE
                qf_s[t0 + u] = q
                for r in range(0, D, 16):
                    qt_s[t0 + u, pl.ds(r // 2, 8), :] = staged_pack(
                        stage_s[1], jnp.concatenate([q[r:r + 16]] * 2, axis=1))[:, :128]

        x0.wait()
        wg.start()
        wu.start()
        project_kv(0)
        x_terms(0, 4)
        project_q(0)
        for d in range(HD):
            spread_q(0, 0, d)
        x1.wait()
        wd.start()
        wo.start()
        for t0 in (4, 8, 12):
            project_kv(t0)
        x_terms(4, NQ)
        project_q(4)
        for i in range(AHEAD):
            if on_vpu[i]:
                for _, piece in vpu_scores(i, stage_s[2]):
                    piece()
        project_q(8)
        vbig_s[pl.ds(0, 8), :] = v_big[0]
        wg.wait()
        wu.wait()
        project_q(12, [functools.partial(gate_up_terms, which, c, r)
                       for c in range(0, 6, 2) for r in range(0, 256, 16) for which in range(2)])
        wd.wait()
        for r in range(0, F // 2, 16):
            blocks = [wd_v[pl.ds(F // 2 * u + r, 16), pl.ds(256 * v, 256)].astype(F32)
                      for u in range(2) for v in range(2)]
            for m, val in enumerate(_strassen_rhs(*blocks)):
                wd_s[m, pl.ds(r // 2, 8), :] = _pack(val)
        wd_rest_s[...] = pltpu.bitcast(wd_v[:, pl.ds(512, 128)], U32)
        wo.wait()
        for c in range(D // 128):
            wo_s[:, pl.ds(128 * c, 128)] = pltpu.bitcast(wo_v[:, pl.ds(128 * c, 128)], U32)

    zero = opaque_zero()
    next_block = jnp.minimum(step + 1, NQ - 1)

    def queued_spread(block, s, d):
        spread_q(block + opaque_zero(), s, d)
        lhs_s[pl.ds(L_SINK, 8), :] = pltpu.bitcast(qb_s[s][pl.ds(opaque_zero(), 8), :], U32)

    queue = []
    for i, (s, t) in enumerate(tiles):
        if on_vpu[i] and i >= AHEAD:
            queue += [(cost, i, piece) for cost, piece in vpu_scores(i, stage_s[0])]
        for d in range(HD):
            if t == (d if s else max(d, AHEAD)):
                where = (step, s + 1) if s + 1 < NS else (next_block, 0)
                queue.append((C_SPREAD, n, functools.partial(queued_spread, *where, d)))
    for i in range(AHEAD):
        if on_vpu[i]:
            queue += [(cost, n, piece) for cost, piece in vpu_scores(i, stage_s[0])]
    capacity = ((300 + 8 * (O_INSIDE + TAIL_SLOTS)) * W_DENSE
                + sum(slots) * W_QK + (n - LAG) * W_PV)
    rate = sum(item[0] for item in queue) / capacity
    credit = [0.0]

    def run_next():
        cost, _, thunk = queue.pop(0)
        credit[0] -= cost
        thunk()

    def paced(load, count, weight):
        rows = []
        for r in range(count):
            credit[0] += weight * rate
            ran = False
            while queue and credit[0] >= queue[0][0] - 1e-6:
                run_next()
                ran = True
            rows.append(load(r, ran))
        return jnp.concatenate(rows, axis=0)

    zeros8 = jnp.zeros((8, TQ), U32)
    sublane = lax.broadcasted_iota(jnp.int32, (8, TQ), 0)
    q_tile, acc, sums = {}, {}, {}

    def q_weights(s):
        base = 40 * s if isinstance(s, int) else pl.multiple_of(40 * s, 8)
        cols = []
        for j in range(HS):
            parts = []
            for r in range(8):
                lo, hi = 10 * j - 8 * r, 10 * j + 10 - 8 * r
                if hi <= 0 or lo >= 8:
                    parts.append(zeros8)
                else:
                    keep = (sublane >= lo) if lo > 0 else (sublane < hi)
                    parts.append(jnp.where(keep, qt_s[step, pl.ds(base + 8 * r, 8), :], zeros8))
            cols.append(jnp.concatenate(parts, axis=0))
        return _unpack(jnp.concatenate(cols, axis=1))

    def scores(i):
        s, t = tiles[i]
        if t == 0:
            q_tile[s] = q_weights(s)
        ordered = lhs_s.at[pl.ds(zero + L_K + 64 * t, 64)]
        free = lhs2_s.at[pl.ds(opaque_zero() + L_K + 64 * t, 64)]
        keys = paced(lambda r, ran: (ordered if ran else free)[pl.ds(8 * r, 8), :], slots[i], W_QK)
        ring_s[i % RING][pl.ds(0, 8 * slots[i]), :] = _pack(jnp.exp2(_dot(_unpack(keys), q_tile[s])))

    def weigh_values(i):
        s, t = tiles[i]
        while any(item[1] <= i for item in queue):
            run_next()
        credit[0] += W_PV * rate
        for j in range(HS):
            p = [ring_s[i % RING][pl.ds(zero, 8 * slots[i]), pl.ds(j * TQ, TQ)]]
            if on_vpu[i]:
                p += [lhs_s[pl.ds(L_P + 64 * i + 32 * u + 8 * j, 8), :] for u in range(2)]
            r = _dot(vt_s[t, pl.ds(24 * (j % 2), 24), :], _unpack(jnp.concatenate(p, axis=0)))
            acc[s, j] = r if t == 0 else r + acc[s, j]

    def normalize(s):
        for j in range(0, HS, 2):
            even, odd = acc.pop((s, j)), acc.pop((s, j + 1))
            total = jnp.where(sublane < 4, odd[0:8], even[16:24])
            sums["min"] = jnp.minimum(sums["min"], total) if sums else total
            sums["all"] = sums["all"] + total if "all" in sums else total
            inv = 1.0 / total
            even = even * jnp.broadcast_to(inv[4:5], (24, TQ))
            odd = odd * jnp.broadcast_to(inv[0:1], (24, TQ))
            ot_s[pl.ds((s * HS + j) * DH, 2 * DH), :] = jnp.concatenate(
                [even[0:16], jnp.where(sublane < 4, even[16:24], odd[0:8]), odd[8:24]], axis=0)

    x_ordered = lhs_s.at[pl.ds(pl.multiple_of(L_X + step * 512, 32), 512)]
    zero_words = lhs_s.at[pl.ds(zero + L_ZERO, 8)]

    def x_rows(bases, count):
        free = lhs2_s.at[pl.ds(pl.multiple_of(L_X + step * 512 + opaque_zero(), 32), 512)]
        return _unpack(paced(lambda r, ran: jnp.concatenate(
            [src[pl.ds(base + 8 * r, 8), :] for src, base in zip((x_ordered, free), bases)], axis=1),
            count, W_DENSE))

    def activation_rows(refs, c0, nc):
        rows = []
        for ref in refs:
            view = ref.at[pl.ds(opaque_zero(), ref.shape[0])]

            def load(r, ran, view=view):
                blk = view[pl.ds(16 * r, 16), pl.ds(c0, nc)]
                if ran:
                    head = blk[0:8, 0:128] + pltpu.bitcast(zero_words[...], F32)
                    blk = jnp.concatenate([jnp.concatenate([head, blk[0:8, 128:]], axis=1), blk[8:]], axis=0)
                return blk

            rows.append(paced(load, ref.shape[0] // 16, W_DENSE))
        return jnp.concatenate(rows, axis=0)

    def park(slot, val):
        park_s[slot][...] = val
        return lambda: park_s[slot][pl.ds(opaque_zero(), 64), :]

    def reglu(gate_up):
        return jnp.maximum(gate_up[:, :128], 0.0) * gate_up[:, 128:]

    def gate_up(c):
        gu_s[...] = _dot(x_rows([448], 8), _unpack(wgu_rest_s[c]))

        def rest(u, v):
            return gu_s[pl.ds(opaque_zero() + 64 * u, 64), pl.ds(256 * v, 256)]

        def product(m):
            return _dot(x_rows([64 * m, 64 * m + 32], 4), _unpack(wgu_s[c, m]))

        m1 = product(0)
        c11 = park(0, m1 + product(6))
        c22 = park(1, m1 + product(5))
        m4 = product(3)
        c11 = park(0, c11() + m4)
        c21 = rest(1, 0) + m4
        m2 = product(1)
        h21 = reglu(c21 + m2)
        c22 = park(1, c22() - m2)
        m5 = product(4)
        h11 = reglu(c11() - m5 + rest(0, 0))
        c12 = rest(0, 1) + m5
        m3 = product(2)
        h12 = reglu(c12 + m3)
        h22 = reglu(c22() + m3 + rest(1, 1))
        for ref, val in zip(h_s, _strassen_lhs(h11, h12, h21, h22) + (h12, h21)):
            ref[:, pl.ds(128 * c, 128)] = val

    def down():
        def product(m):
            r = None
            for u in range(3):
                term = _dot(activation_rows([h_s[m]], 256 * u, 256), _unpack(wd_s[m, pl.ds(128 * u, 128), :]))
                r = term if r is None else term + r
            return r

        m1 = park(0, product(0))
        m6 = product(5)
        c22 = park(1, m1() + m6)
        m7 = product(6)
        c11 = park(0, m1() + m7)
        m4 = product(3)
        c11 = park(0, c11() + m4)
        c21 = park(2, m4)
        m2 = product(1)
        b_s[0][pl.ds(64, 64), pl.ds(0, 256)] = c21() + m2
        c22 = park(1, c22() - m2)
        m5 = product(4)
        b_s[0][pl.ds(0, 64), pl.ds(0, 256)] = c11() - m5
        c12 = park(2, m5)
        m3 = product(2)
        b_s[0][pl.ds(0, 64), pl.ds(256, 256)] = c12() + m3
        b_s[0][pl.ds(64, 64), pl.ds(256, 256)] = c22() + m3

    def down_rest(u):
        left = activation_rows([h_s[2], h_s[8]], 256 * u, 256)
        right = jnp.concatenate([h_s[m][pl.ds(opaque_zero(), 64), pl.ds(256 * u, 256)] for m in (7, 3)], axis=0)
        w = jnp.concatenate([wd_rest_s[pl.ds(384 * v + 128 * u, 128), :] for v in range(2)], axis=0)
        r = _dot(jnp.concatenate([left, right], axis=1), _unpack(w))
        b_s[1][...] = r if u == 0 else b_s[1][pl.ds(opaque_zero(), TQ), :] + r

    def wo_tile(r0, nr, c0, nc):
        return _unpack(wo_s[pl.ds(r0 // 2, nr // 2), pl.ds(c0, nc)])

    def out_proj(c):
        a_s[:, pl.ds(128 * c, 128)] = _dot(activation_rows([o_s], 0, 512), wo_tile(0, 512, 128 * c, 128))

    def mix(a, which):
        g = jnp.concatenate([g_s[pl.ds(pl.multiple_of(step * TQ, TQ), TQ), :]] * (a.shape[1] // 128), axis=1)
        b = b_s[which][pl.ds(opaque_zero(), TQ), :]
        out_ref[:, pl.ds(512 * which, a.shape[1])] = (g * a + (1.0 - g) * b).astype(out_ref.dtype)

    for c in range(6):
        gate_up(c)
    rest_jobs = [functools.partial(down_rest, u) for u in range(3)]
    out_jobs = [functools.partial(out_proj, c) for c in range(O_INSIDE, D // 128)]
    tail = out_jobs + rest_jobs if O_FIRST else rest_jobs + out_jobs
    o_tile_done = {2: 0, 4: 1, 5: 2, 7: 3}
    for i in range(n + LAG):
        if i == DOWN_AT:
            down()
        if i < n:
            scores(i)
        else:
            tail.pop(0)()
        if i >= LAG:
            s, t = tiles[i - LAG]
            weigh_values(i - LAG)
            if t == 2 and s > 0:
                normalize(s - 1)
                if s in o_tile_done:
                    k = 128 * o_tile_done[s]
                    o_s[:, pl.ds(k, 128)] = ot_s[pl.ds(opaque_zero() + k, 128), :].T
            if s == NS - 1 and t in range(4, 4 + 2 * O_INSIDE, 2):
                out_proj((t - 4) // 2)
    normalize(NS - 1)
    for job in tail:
        job()
    while queue:
        run_next()
    o_last = ot_s[pl.ds(opaque_zero() + 512, 128), :].T
    mix(a_s[pl.ds(opaque_zero(), TQ), pl.ds(0, 512)] + _dot(o_last, wo_tile(512, 128, 0, 512)), 0)
    w_last = wo_tile(512, 128, 512, 128)
    mix(a_s[pl.ds(opaque_zero(), TQ), pl.ds(512, 128)]
        + jnp.concatenate([_dot(o_last[32 * r:32 * r + 32], w_last) for r in range(4)], axis=0), 1)

    safe = (sums["min"] >= SUM_MIN) & (sums["all"] <= SUM_MAX) & (vbig_s[pl.ds(0, 8), :] == 0.0)

    @pl.when(jnp.max(jnp.where(safe, 0.0, 1.0)) > 0.0)
    def _redo_with_true_max():
        def slab(s, carry):
            w = q_weights(s)

            def tile_scores(t):
                return _dot(_unpack(lhs_s[pl.ds(pl.multiple_of(L_K + 64 * t, 64), 64), :]), w)

            row_max = lax.fori_loop(
                0, NT, lambda t, m: jnp.maximum(m, jnp.max(tile_scores(t), axis=0, keepdims=True)),
                jnp.full((1, HS * TQ), -jnp.inf, F32))
            o = lax.fori_loop(
                0, NT, lambda t, o: o + _dot(vt_s[t, pl.ds(0, 24), :], jnp.exp2(tile_scores(t) - row_max)),
                jnp.zeros((24, HS * TQ), F32))
            o = o * (1.0 / o[DH:DH + 1])
            ot_s[pl.ds(pl.multiple_of(s * HS * DH, 8), HS * DH), :] = jnp.concatenate(
                [o[:DH, j * TQ:(j + 1) * TQ] for j in range(HS)], axis=0)
            return carry

        lax.fori_loop(0, NS, slab, 0)
        a = _dot(ot_s[...].T, wo_tile(0, D, 0, D))
        mix(a[:, :512], 0)
        mix(a[:, 512:], 1)


@jax.jit
def pallas_gated_mix__grouped_kv_mqa__glu_gated_reglu__prompt_kernel(
    A_x: jax.Array,
    A_wq: jax.Array,
    A_wk: jax.Array,
    A_wv: jax.Array,
    A_wo: jax.Array,
    B_x: jax.Array,
    B_W_gate: jax.Array,
    B_W_up: jax.Array,
    B_W_down: jax.Array,
    gate_w: jax.Array,
):
    del B_x
    vmem = pltpu.VMEM
    scratch = [
        vmem((S, D), BF16), vmem((D, D), BF16), vmem((D, F), BF16), vmem((D, F), BF16),
        vmem((F, D), BF16), vmem((D, D), BF16),
        vmem((D // 2 + 32, D), U32),
        vmem((4, D, 128), F32),
        vmem((L_ROWS, 128), U32),
        vmem((L_ZERO, 128), U32),
        vmem((NT * TERM_ROWS, 128), F32),
        vmem((NQ, D // 2, TQ), U32),
        vmem((NQ, D, TQ), F32),
        vmem((NT, 48, 128), F32),
        vmem((S, 128), F32),
        vmem((6, 7, 128, 256), U32),
        vmem((6, 64, 512), U32),
        vmem((7, F // 4, 256), U32),
        vmem((F // 2, 128), U32),
        vmem((D // 2, D), U32),
        vmem((D, TQ), F32),
        vmem((TQ, 512), F32),
        vmem((TQ, D), F32),
        vmem((TQ, 512), F32),
        vmem((32, 128), F32),
        [vmem((64, HS * TQ), U32)] * RING,
        [vmem((TERM_ROWS, TQ), F32)] * NS,
        [vmem((TQ, 512), F32), vmem((TQ, 128), F32)],
        [vmem((64, F // 2), F32)] * 9,
        [vmem((64, 256), F32)] * 3,
        [vmem((8, 256), U32)] * 3,
        vmem((2, DH, D), BF16),
        vmem((D,), BF16),
        pltpu.SemaphoreType.DMA((10,)),
    ]
    out = pl.pallas_call(
        _kernel,
        grid=(NQ,),
        in_specs=[pl.BlockSpec(memory_space=pl.ANY)] * 9,
        out_specs=pl.BlockSpec((TQ, D), lambda i: (i, 0)),
        out_shape=jax.ShapeDtypeStruct((S, D), A_x.dtype),
        scratch_shapes=scratch,
        compiler_params=pltpu.CompilerParams(
            dimension_semantics=("arbitrary",), vmem_limit_bytes=100 * 2 ** 20),
    )(A_x.reshape(S, D), A_wq, A_wk.T, A_wv.T, gate_w, B_W_gate, B_W_up, B_W_down, A_wo)
    return out.reshape(1, S, D)
```

```python
import functools
import math

import jax
import jax.experimental.pallas as pl
import jax.experimental.pallas.tpu as pltpu
import jax.numpy as jnp
from jax import lax

S, D, H, DH, F = 2048, 640, 32, 20, 1536
TQ = 128
NQ = S // TQ
HS = 4
NS = H // HS
NT = S // 128
HD = DH // 2
X_FIRST = 512
BF16, F32, U32 = jnp.bfloat16, jnp.float32, jnp.uint32
Q_SCALE = DH ** -0.5 * math.log2(math.e)

SUM_MIN, SUM_MAX, V_MAX = 2.0 ** -20, 2.0 ** 90, 2.0 ** 30

VPU_TILES = 111
AHEAD = 3
LAG = 3
RING = LAG + 1
DOWN_AT = 2
O_INSIDE = 2
O_FIRST = 1
TAIL_SLOTS = 5.5
W_DENSE, W_QK, W_PV = 54, 52, 100
C_SPREAD = 40

L_K = 0
L_X = L_K + S // 2
L_ZERO = L_X + NQ * 512
L_SINK = L_ZERO + 32
L_P = L_SINK + 32
L_ROWS = L_P + NS * NT * 64
TERM_ROWS = 7 * HD * 16


def _dot(a, b):
    return lax.dot_general(a, b, (((1,), (0,)), ((), ())), preferred_element_type=F32)


def _dot_nt(a, b):
    return lax.dot_general(a, b, (((1,), (1,)), ((), ())), preferred_element_type=F32)


def _pack(val):
    return pltpu.bitcast(val.astype(BF16), U32)


def _unpack(words):
    return pltpu.bitcast(words, BF16)


def _strassen_lhs(a11, a12, a21, a22):
    return a11 + a22, a21 + a22, a11, a22, a11 + a12, a21 - a11, a12 - a22


def _strassen_rhs(b11, b12, b21, b22):
    return b11 + b22, b11, b12 - b22, b21 - b11, b22, b11 + b12, b21 + b22


def _winograd_lhs(a11, a12, a21, a22):
    s1 = a21 + a22
    s2 = s1 - a11
    return a11, a12, a12 - s2, a22, s1, s2, a11 - a21


def _winograd_rhs(b11, b12, b21, b22):
    t1 = b12 - b11
    t2 = b22 - t1
    return b11, b21, b22, b21 - t2, t1, t2, b22 - b12


def _kernel(x_hbm, wq_hbm, wk_hbm, wv_hbm, gw_hbm, wg_hbm, wu_hbm, wd_hbm, wo_hbm, out_ref,
            x_v, wq_v, wg_v, wu_v, wd_v, wo_v,
            wqt_s, qpart_s, lhs_s, lhs2_s, kb_s, qt_s, qf_s, vt_s, g_s,
            wgu_s, wgu_rest_s, wd_s, wd_rest_s, wo_s,
            ot_s, o_s, a_s, gu_s, vbig_s, ring_s, qb_s, b_s, h_s, park_s, stage_s,
            wkv_v, gw_v, sems):
    step = pl.program_id(0)
    tiles = [(s, t) for s in range(NS) for t in range(NT)]
    n = len(tiles)
    on_vpu = [(n - i) * VPU_TILES // n > (n - i - 1) * VPU_TILES // n for i in range(n)]
    slots = [6 if v else 8 for v in on_vpu]
    n_zero = [0]

    def opaque_zero():
        n_zero[0] += 1
        return pl.multiple_of(((step + n_zero[0]) >> 16) * 32, 32)

    def staged_pack(stage, val):
        stage[...] = _pack(val)
        return stage[...]

    def spread_q(block, s, d):
        for c in range(2):
            b11, b21, b12, b22 = [
                jnp.broadcast_to(qf_s[block, pl.ds(DH * (HS * s + c + 2 * u) + HD * v + d, 1), :], (8, TQ))
                for u in range(2) for v in range(2)]
            for m, val in enumerate(_winograd_rhs(b11, b12, b21, b22)):
                qb_s[s][pl.ds((m * HD + d) * 16 + 8 * c, 8), :] = val

    def vpu_scores(i, stage):
        s, t = tiles[i]
        live = {}

        def product(m, acc):
            zero = opaque_zero()
            rows = pl.ds(m * HD * 16, HD * 16)
            q = qb_s[s].at[pl.ds(zero, TERM_ROWS)][rows, :].reshape(HD, 16, TQ)
            k = kb_s.at[pl.ds(zero + t * TERM_ROWS, TERM_ROWS)][rows, :]
            q = jnp.concatenate([q[:, :8], q[:, 8:]], axis=2)
            q = jnp.concatenate([q, q], axis=1).reshape(HD * 16, 2 * TQ)
            k = jnp.concatenate([k, k], axis=1)
            for kd, qd in zip(jnp.split(k, HD), jnp.split(q, HD)):
                acc = kd * qd if acc is None else acc + kd * qd
            return acc

        def emit(scores, u, j):
            p = staged_pack(stage, jnp.exp2(scores))
            for c in range(2):
                lhs_s[pl.ds(L_P + 64 * i + 32 * u + 8 * (j + c), 8), :] = p[:, c * TQ:(c + 1) * TQ]

        def c11():
            live["m1"] = product(0, None)
            emit(product(1, live["m1"]), 0, 0)

        def c12():
            live["u2"] = product(5, live.pop("m1"))
            live["m5"] = product(4, None)
            emit(product(2, live["u2"] + live["m5"]), 0, 2)

        def c22():
            live["u3"] = product(6, live.pop("u2"))
            emit(live["u3"] + live.pop("m5"), 1, 2)

        def c21():
            emit(product(3, live.pop("u3")), 1, 0)

        return [(162, c11), (246, c12), (90, c22), (86, c21)]

    @pl.when(step == 0)
    def _load_and_project():
        first, rest = pl.ds(0, X_FIRST), pl.ds(X_FIRST, S - X_FIRST)
        wq, wk, wv, gw, x0, x1, wg, wu, wd, wo = [
            pltpu.make_async_copy(src, dst, sems.at[i]) for i, (src, dst) in enumerate((
                (wq_hbm, wq_v), (wk_hbm, wkv_v.at[0]), (wv_hbm, wkv_v.at[1]), (gw_hbm, gw_v),
                (x_hbm.at[first, :], x_v.at[first, :]), (x_hbm.at[rest, :], x_v.at[rest, :]),
                (wg_hbm, wg_v), (wu_hbm, wu_v), (wd_hbm, wd_v), (wo_hbm, wo_v)))]
        for copy in (wq, wk, wv, gw, x0, x1):
            copy.start()
        lhs_s[pl.ds(L_ZERO, 8), :] = jnp.zeros((8, 128), U32)
        for copy in (wq, wk, wv, gw):
            copy.wait()
        wkv = jnp.concatenate(
            [wkv_v[0].astype(F32), jnp.broadcast_to(gw_v[...].astype(F32).reshape(1, D), (8, D)),
             wkv_v[1].astype(F32)], axis=0).astype(BF16)
        wqt_s[pl.ds(0, D // 2), :] = pltpu.bitcast(wq_v[...].T, U32)
        lane = lax.broadcasted_iota(jnp.int32, (64, 128), 1)
        row = lax.broadcasted_iota(jnp.int32, (24, 128), 0)
        v_big = [jnp.zeros((8, 128), F32)]

        def project_kv(t0):
            kv = _dot_nt(wkv, x_v[pl.ds(128 * t0, 512), :])
            for t in range(t0, t0 + 4):
                kvt = kv[:, 128 * (t - t0):128 * (t - t0 + 1)]
                v_odd = jnp.where(row < 4, 1.0, kvt[24:48])
                vt_s[t, pl.ds(24, 24), :] = v_odd
                vt_s[t, pl.ds(0, 24), :] = jnp.concatenate([v_odd[4:24], jnp.ones((4, 128), F32)], axis=0)
                for r in range(3):
                    v_big[0] = jnp.where(jnp.abs(v_odd[8 * r:8 * r + 8]) <= V_MAX, v_big[0], 1.0)
                k = jnp.concatenate([kvt[0:DH]] * HS + [jnp.zeros((120 - HS * DH, 128), F32),
                                                        jax.nn.sigmoid(kvt[16:24])], axis=0).T
                g_s[pl.ds(128 * t, 128), :] = jnp.broadcast_to(k[:, 124:125], (128, 128))
                words = jnp.where(lane < HS * DH, _pack(k), jnp.zeros((64, 128), U32))
                lhs_s[pl.ds(L_K + 64 * t, 64), :] = words
                lhs2_s[pl.ds(L_K + 64 * t, 64), :] = words
                for d in range(HD):
                    lo = jnp.broadcast_to(k[96:, d:d + 1], (32, 128))
                    hi = jnp.broadcast_to(k[96:, HD + d:HD + d + 1], (32, 128))
                    for m, val in enumerate(_winograd_lhs(lo[:16], hi[:16], lo[16:], hi[16:])):
                        kb_s[pl.ds(t * TERM_ROWS + (m * HD + d) * 16, 16), :] = val

        def x_terms(t0, t1):
            for t in range(t0, t1):
                for r in range(0, 64, 16):
                    blocks = [x_v[pl.ds(128 * t + 64 * u + r, 16), pl.ds(256 * v, 256)].astype(F32)
                              for u in range(2) for v in range(2)]
                    for m, val in enumerate(_strassen_lhs(*blocks)):
                        val = staged_pack(stage_s[1], val)
                        for u, dst in enumerate((lhs_s, lhs2_s)):
                            dst[pl.ds(L_X + 512 * t + 64 * m + 32 * u + r // 2, 8), :] = (
                                val[:, 128 * u:128 * (u + 1)])
                    lhs_s[pl.ds(L_X + 512 * t + 448 + r, 16), :] = pltpu.bitcast(
                        x_v[pl.ds(128 * t + 2 * r, 32), pl.ds(512, 128)], U32)

        def gate_up_terms(which, c, r):
            w = (wg_v, wu_v)[which]
            blocks = [w[pl.ds(256 * u + r, 16), pl.ds(128 * (c + 6 * v), 256)].astype(F32)
                      for u in range(2) for v in range(2)]
            for m, val in enumerate(_strassen_rhs(*blocks)):
                val = staged_pack(stage_s[1], val)
                for u in range(2):
                    wgu_s[c + u, m, pl.ds(r // 2, 8), pl.ds(128 * which, 128)] = val[:, 128 * u:128 * (u + 1)]
            if r < 128:
                for v in range(2):
                    val = staged_pack(stage_s[1], w[pl.ds(512 + r, 16), pl.ds(128 * (c + 6 * v), 256)].astype(F32))
                    for u in range(2):
                        wgu_rest_s[c + u, pl.ds(r // 2, 8), pl.ds(256 * v + 128 * which, 128)] = (
                            val[:, 128 * u:128 * (u + 1)])
            wqt_s[pl.ds(D // 2, 8), pl.ds(0, 128)] = wgu_s[c, 0, pl.ds(opaque_zero(), 8), pl.ds(0, 128)]

        def project_q(t0, work=()):
            def lhs(c0, nc, part):
                per = len(work) / (4 * D // 16)
                view = wqt_s.at[pl.ds(opaque_zero(), D // 2)]
                rows = []
                for r in range(D // 16):
                    if part is not None:
                        at = part * D // 16 + r
                        for item in work[int(at * per):int((at + 1) * per)]:
                            item()
                    rows.append(view[pl.ds(8 * r, 8), pl.ds(c0, nc)])
                return _unpack(jnp.concatenate(rows, axis=0))

            q_rest = _dot_nt(lhs(512, 128, None), x_v[pl.ds(128 * t0, 512), pl.ds(512, 128)])
            for u in range(4):
                qpart_s[u] = q_rest[:, 128 * u:128 * (u + 1)]
            for u in range(4):
                q = qpart_s[u, pl.ds(opaque_zero(), D), :] + _dot_nt(
                    lhs(0, 512, u), x_v[pl.ds(128 * (t0 + u), 128), pl.ds(0, 512)])
                q = q * Q_SCALE
                qf_s[t0 + u] = q
                for r in range(0, D, 16):
                    qt_s[t0 + u, pl.ds(r // 2, 8), :] = staged_pack(
                        stage_s[1], jnp.concatenate([q[r:r + 16]] * 2, axis=1))[:, :128]

        x0.wait()
        wg.start()
        wu.start()
        project_kv(0)
        x_terms(0, 4)
        project_q(0)
        for d in range(HD):
            spread_q(0, 0, d)
        x1.wait()
        wd.start()
        wo.start()
        for t0 in (4, 8, 12):
            project_kv(t0)
        x_terms(4, NQ)
        project_q(4)
        for i in range(AHEAD):
            if on_vpu[i]:
                for _, piece in vpu_scores(i, stage_s[2]):
                    piece()
        project_q(8)
        vbig_s[pl.ds(0, 8), :] = v_big[0]
        wg.wait()
        wu.wait()
        project_q(12, [functools.partial(gate_up_terms, which, c, r)
                       for c in range(0, 6, 2) for r in range(0, 256, 16) for which in range(2)])
        wd.wait()
        for r in range(0, F // 2, 16):
            blocks = [wd_v[pl.ds(F // 2 * u + r, 16), pl.ds(256 * v, 256)].astype(F32)
                      for u in range(2) for v in range(2)]
            for m, val in enumerate(_strassen_rhs(*blocks)):
                wd_s[m, pl.ds(r // 2, 8), :] = _pack(val)
        wd_rest_s[...] = pltpu.bitcast(wd_v[:, pl.ds(512, 128)], U32)
        wo.wait()
        for c in range(D // 128):
            wo_s[:, pl.ds(128 * c, 128)] = pltpu.bitcast(wo_v[:, pl.ds(128 * c, 128)], U32)

    zero = opaque_zero()
    next_block = jnp.minimum(step + 1, NQ - 1)

    def queued_spread(block, s, d):
        spread_q(block + opaque_zero(), s, d)
        lhs_s[pl.ds(L_SINK, 8), :] = pltpu.bitcast(qb_s[s][pl.ds(opaque_zero(), 8), :], U32)

    queue = []
    for i, (s, t) in enumerate(tiles):
        if on_vpu[i] and i >= AHEAD:
            queue += [(cost, i, piece) for cost, piece in vpu_scores(i, stage_s[0])]
        for d in range(HD):
            if t == (d if s else max(d, AHEAD)):
                where = (step, s + 1) if s + 1 < NS else (next_block, 0)
                queue.append((C_SPREAD, n, functools.partial(queued_spread, *where, d)))
    for i in range(AHEAD):
        if on_vpu[i]:
            queue += [(cost, n, piece) for cost, piece in vpu_scores(i, stage_s[0])]
    capacity = ((300 + 8 * (O_INSIDE + TAIL_SLOTS)) * W_DENSE
                + sum(slots) * W_QK + (n - LAG) * W_PV)
    rate = sum(item[0] for item in queue) / capacity
    credit = [0.0]

    def run_next():
        cost, _, thunk = queue.pop(0)
        credit[0] -= cost
        thunk()

    def paced(load, count, weight):
        rows = []
        for r in range(count):
            credit[0] += weight * rate
            ran = False
            while queue and credit[0] >= queue[0][0] - 1e-6:
                run_next()
                ran = True
            rows.append(load(r, ran))
        return jnp.concatenate(rows, axis=0)

    zeros8 = jnp.zeros((8, TQ), U32)
    sublane = lax.broadcasted_iota(jnp.int32, (8, TQ), 0)
    q_tile, acc, sums = {}, {}, {}

    def q_weights(s):
        base = 40 * s if isinstance(s, int) else pl.multiple_of(40 * s, 8)
        cols = []
        for j in range(HS):
            parts = []
            for r in range(8):
                lo, hi = 10 * j - 8 * r, 10 * j + 10 - 8 * r
                if hi <= 0 or lo >= 8:
                    parts.append(zeros8)
                else:
                    keep = (sublane >= lo) if lo > 0 else (sublane < hi)
                    parts.append(jnp.where(keep, qt_s[step, pl.ds(base + 8 * r, 8), :], zeros8))
            cols.append(jnp.concatenate(parts, axis=0))
        return _unpack(jnp.concatenate(cols, axis=1))

    def scores(i):
        s, t = tiles[i]
        if t == 0:
            q_tile[s] = q_weights(s)
        ordered = lhs_s.at[pl.ds(zero + L_K + 64 * t, 64)]
        free = lhs2_s.at[pl.ds(opaque_zero() + L_K + 64 * t, 64)]
        keys = paced(lambda r, ran: (ordered if ran else free)[pl.ds(8 * r, 8), :], slots[i], W_QK)
        ring_s[i % RING][pl.ds(0, 8 * slots[i]), :] = _pack(jnp.exp2(_dot(_unpack(keys), q_tile[s])))

    def weigh_values(i):
        s, t = tiles[i]
        while any(item[1] <= i for item in queue):
            run_next()
        credit[0] += W_PV * rate
        for j in range(HS):
            p = [ring_s[i % RING][pl.ds(zero, 8 * slots[i]), pl.ds(j * TQ, TQ)]]
            if on_vpu[i]:
                p += [lhs_s[pl.ds(L_P + 64 * i + 32 * u + 8 * j, 8), :] for u in range(2)]
            r = _dot(vt_s[t, pl.ds(24 * (j % 2), 24), :], _unpack(jnp.concatenate(p, axis=0)))
            acc[s, j] = r if t == 0 else r + acc[s, j]

    def normalize(s):
        for j in range(0, HS, 2):
            even, odd = acc.pop((s, j)), acc.pop((s, j + 1))
            total = jnp.where(sublane < 4, odd[0:8], even[16:24])
            sums["min"] = jnp.minimum(sums["min"], total) if sums else total
            sums["all"] = sums["all"] + total if "all" in sums else total
            inv = 1.0 / total
            even = even * jnp.broadcast_to(inv[4:5], (24, TQ))
            odd = odd * jnp.broadcast_to(inv[0:1], (24, TQ))
            ot_s[pl.ds((s * HS + j) * DH, 2 * DH), :] = jnp.concatenate(
                [even[0:16], jnp.where(sublane < 4, even[16:24], odd[0:8]), odd[8:24]], axis=0)

    x_ordered = lhs_s.at[pl.ds(pl.multiple_of(L_X + step * 512, 32), 512)]
    zero_words = lhs_s.at[pl.ds(zero + L_ZERO, 8)]

    def x_rows(bases, count):
        free = lhs2_s.at[pl.ds(pl.multiple_of(L_X + step * 512 + opaque_zero(), 32), 512)]
        return _unpack(paced(lambda r, ran: jnp.concatenate(
            [src[pl.ds(base + 8 * r, 8), :] for src, base in zip((x_ordered, free), bases)], axis=1),
            count, W_DENSE))

    def activation_rows(refs, c0, nc):
        rows = []
        for ref in refs:
            view = ref.at[pl.ds(opaque_zero(), ref.shape[0])]

            def load(r, ran, view=view):
                blk = view[pl.ds(16 * r, 16), pl.ds(c0, nc)]
                if ran:
                    head = blk[0:8, 0:128] + pltpu.bitcast(zero_words[...], F32)
                    blk = jnp.concatenate([jnp.concatenate([head, blk[0:8, 128:]], axis=1), blk[8:]], axis=0)
                return blk

            rows.append(paced(load, ref.shape[0] // 16, W_DENSE))
        return jnp.concatenate(rows, axis=0)

    def park(slot, val):
        park_s[slot][...] = val
        return lambda: park_s[slot][pl.ds(opaque_zero(), 64), :]

    def reglu(gate_up):
        return jnp.maximum(gate_up[:, :128], 0.0) * gate_up[:, 128:]

    def gate_up(c):
        gu_s[...] = _dot(x_rows([448], 8), _unpack(wgu_rest_s[c]))

        def rest(u, v):
            return gu_s[pl.ds(opaque_zero() + 64 * u, 64), pl.ds(256 * v, 256)]

        def product(m):
            return _dot(x_rows([64 * m, 64 * m + 32], 4), _unpack(wgu_s[c, m]))

        m1 = product(0)
        c11 = park(0, m1 + product(6))
        c22 = park(1, m1 + product(5))
        m4 = product(3)
        c11 = park(0, c11() + m4)
        c21 = rest(1, 0) + m4
        m2 = product(1)
        h21 = reglu(c21 + m2)
        c22 = park(1, c22() - m2)
        m5 = product(4)
        h11 = reglu(c11() - m5 + rest(0, 0))
        c12 = rest(0, 1) + m5
        m3 = product(2)
        h12 = reglu(c12 + m3)
        h22 = reglu(c22() + m3 + rest(1, 1))
        for ref, val in zip(h_s, _strassen_lhs(h11, h12, h21, h22) + (h12, h21)):
            ref[:, pl.ds(128 * c, 128)] = val

    def down():
        def product(m):
            r = None
            for u in range(3):
                term = _dot(activation_rows([h_s[m]], 256 * u, 256), _unpack(wd_s[m, pl.ds(128 * u, 128), :]))
                r = term if r is None else term + r
            return r

        m1 = park(0, product(0))
        m6 = product(5)
        c22 = park(1, m1() + m6)
        m7 = product(6)
        c11 = park(0, m1() + m7)
        m4 = product(3)
        c11 = park(0, c11() + m4)
        c21 = park(2, m4)
        m2 = product(1)
        b_s[0][pl.ds(64, 64), pl.ds(0, 256)] = c21() + m2
        c22 = park(1, c22() - m2)
        m5 = product(4)
        b_s[0][pl.ds(0, 64), pl.ds(0, 256)] = c11() - m5
        c12 = park(2, m5)
        m3 = product(2)
        b_s[0][pl.ds(0, 64), pl.ds(256, 256)] = c12() + m3
        b_s[0][pl.ds(64, 64), pl.ds(256, 256)] = c22() + m3

    def down_rest(u):
        left = activation_rows([h_s[2], h_s[8]], 256 * u, 256)
        right = jnp.concatenate([h_s[m][pl.ds(opaque_zero(), 64), pl.ds(256 * u, 256)] for m in (7, 3)], axis=0)
        w = jnp.concatenate([wd_rest_s[pl.ds(384 * v + 128 * u, 128), :] for v in range(2)], axis=0)
        r = _dot(jnp.concatenate([left, right], axis=1), _unpack(w))
        b_s[1][...] = r if u == 0 else b_s[1][pl.ds(opaque_zero(), TQ), :] + r

    def wo_tile(r0, nr, c0, nc):
        return _unpack(wo_s[pl.ds(r0 // 2, nr // 2), pl.ds(c0, nc)])

    def out_proj(c):
        a_s[:, pl.ds(128 * c, 128)] = _dot(activation_rows([o_s], 0, 512), wo_tile(0, 512, 128 * c, 128))

    def mix(a, which):
        g = jnp.concatenate([g_s[pl.ds(pl.multiple_of(step * TQ, TQ), TQ), :]] * (a.shape[1] // 128), axis=1)
        b = b_s[which][pl.ds(opaque_zero(), TQ), :]
        out_ref[:, pl.ds(512 * which, a.shape[1])] = (g * a + (1.0 - g) * b).astype(out_ref.dtype)

    for c in range(6):
        gate_up(c)
    rest_jobs = [functools.partial(down_rest, u) for u in range(3)]
    out_jobs = [functools.partial(out_proj, c) for c in range(O_INSIDE, D // 128)]
    tail = out_jobs + rest_jobs if O_FIRST else rest_jobs + out_jobs
    o_tile_done = {2: 0, 4: 1, 5: 2, 7: 3}
    for i in range(n + LAG):
        if i == DOWN_AT:
            down()
        if i < n:
            scores(i)
        else:
            tail.pop(0)()
        if i >= LAG:
            s, t = tiles[i - LAG]
            weigh_values(i - LAG)
            if t == 2 and s > 0:
                normalize(s - 1)
                if s in o_tile_done:
                    k = 128 * o_tile_done[s]
                    o_s[:, pl.ds(k, 128)] = ot_s[pl.ds(opaque_zero() + k, 128), :].T
            if s == NS - 1 and t in range(4, 4 + 2 * O_INSIDE, 2):
                out_proj((t - 4) // 2)
    normalize(NS - 1)
    for job in tail:
        job()
    while queue:
        run_next()
    o_last = ot_s[pl.ds(opaque_zero() + 512, 128), :].T
    mix(a_s[pl.ds(opaque_zero(), TQ), pl.ds(0, 512)] + _dot(o_last, wo_tile(512, 128, 0, 512)), 0)
    w_last = wo_tile(512, 128, 512, 128)
    mix(a_s[pl.ds(opaque_zero(), TQ), pl.ds(512, 128)]
        + jnp.concatenate([_dot(o_last[32 * r:32 * r + 32], w_last) for r in range(4)], axis=0), 1)

    safe = (sums["min"] >= SUM_MIN) & (sums["all"] <= SUM_MAX) & (vbig_s[pl.ds(0, 8), :] == 0.0)

    @pl.when(jnp.max(jnp.where(safe, 0.0, 1.0)) > 0.0)
    def _redo_with_true_max():
        def slab(s, carry):
            w = q_weights(s)

            def tile_scores(t):
                return _dot(_unpack(lhs_s[pl.ds(opaque_zero() + L_K + 128 * t, 128), :]), w)

            row_max = functools.reduce(jnp.maximum, [
                jnp.max(tile_scores(t).reshape(32, 8, HS * TQ), axis=0) for t in range(NT // 2)])
            row_max = jnp.max(row_max, axis=0, keepdims=True)
            p, o = {}, 0.0
            for t in range(NT // 2 + 2):
                if t < NT // 2:
                    p[t] = jnp.exp2(tile_scores(t) - row_max).astype(BF16)
                if t >= 2:
                    v = jnp.concatenate([vt_s[2 * (t - 2) + u, pl.ds(0, 24), :] for u in range(2)], axis=1)
                    o = o + _dot(v, p.pop(t - 2))
            o = o * (1.0 / o[DH:DH + 1])
            ot_s[pl.ds(pl.multiple_of(s * HS * DH, 8), HS * DH), :] = jnp.concatenate(
                [o[:DH, j * TQ:(j + 1) * TQ] for j in range(HS)], axis=0)
            return carry

        lax.fori_loop(0, NS, slab, 0)
        a = _dot(ot_s[...].T, wo_tile(0, D, 0, D))
        mix(a[:, :512], 0)
        mix(a[:, 512:], 1)


@jax.jit
def pallas_gated_mix__grouped_kv_mqa__glu_gated_reglu__prompt_kernel(
    A_x: jax.Array,
    A_wq: jax.Array,
    A_wk: jax.Array,
    A_wv: jax.Array,
    A_wo: jax.Array,
    B_x: jax.Array,
    B_W_gate: jax.Array,
    B_W_up: jax.Array,
    B_W_down: jax.Array,
    gate_w: jax.Array,
):
    del B_x
    vmem = pltpu.VMEM
    scratch = [
        vmem((S, D), BF16), vmem((D, D), BF16), vmem((D, F), BF16), vmem((D, F), BF16),
        vmem((F, D), BF16), vmem((D, D), BF16),
        vmem((D // 2 + 32, D), U32),
        vmem((4, D, 128), F32),
        vmem((L_ROWS, 128), U32),
        vmem((L_ZERO, 128), U32),
        vmem((NT * TERM_ROWS, 128), F32),
        vmem((NQ, D // 2, TQ), U32),
        vmem((NQ, D, TQ), F32),
        vmem((NT, 48, 128), F32),
        vmem((S, 128), F32),
        vmem((6, 7, 128, 256), U32),
        vmem((6, 64, 512), U32),
        vmem((7, F // 4, 256), U32),
        vmem((F // 2, 128), U32),
        vmem((D // 2, D), U32),
        vmem((D, TQ), F32),
        vmem((TQ, 512), F32),
        vmem((TQ, D), F32),
        vmem((TQ, 512), F32),
        vmem((32, 128), F32),
        [vmem((64, HS * TQ), U32)] * RING,
        [vmem((TERM_ROWS, TQ), F32)] * NS,
        [vmem((TQ, 512), F32), vmem((TQ, 128), F32)],
        [vmem((64, F // 2), F32)] * 9,
        [vmem((64, 256), F32)] * 3,
        [vmem((8, 256), U32)] * 3,
        vmem((2, DH, D), BF16),
        vmem((D,), BF16),
        pltpu.SemaphoreType.DMA((10,)),
    ]
    out = pl.pallas_call(
        _kernel,
        grid=(NQ,),
        in_specs=[pl.BlockSpec(memory_space=pl.ANY)] * 9,
        out_specs=pl.BlockSpec((TQ, D), lambda i: (i, 0)),
        out_shape=jax.ShapeDtypeStruct((S, D), A_x.dtype),
        scratch_shapes=scratch,
        compiler_params=pltpu.CompilerParams(
            dimension_semantics=("arbitrary",), vmem_limit_bytes=100 * 2 ** 20),
    )(A_x.reshape(S, D), A_wq, A_wk.T, A_wv.T, gate_w, B_W_gate, B_W_up, B_W_down, A_wo)
    return out.reshape(1, S, D)
```

```python
import functools
import math

import jax
import jax.experimental.pallas as pl
import jax.experimental.pallas.tpu as pltpu
import jax.numpy as jnp
from jax import lax

S, D, H, DH, F = 2048, 640, 32, 20, 1536
TQ = 128
NQ = S // TQ
HS = 4
NS = H // HS
NT = S // 128
HD = DH // 2
X_FIRST = 512
BF16, F32, U32 = jnp.bfloat16, jnp.float32, jnp.uint32
Q_SCALE = DH ** -0.5 * math.log2(math.e)

SUM_MIN, SUM_MAX, V_MAX = 2.0 ** -20, 2.0 ** 90, 2.0 ** 30

VPU_TILES = 111
AHEAD = 3
LAG = 3
RING = LAG + 1
DOWN_AT = 2
O_INSIDE = 2
O_FIRST = 1
TAIL_SLOTS = 5.5
W_DENSE, W_QK, W_PV = 54, 52, 100
C_SPREAD = 40

L_K = 0
L_X = L_K + S // 2
L_ZERO = L_X + NQ * 512
L_SINK = L_ZERO + 32
L_P = L_SINK + 32
L_ROWS = L_P + NS * NT * 64


def _dot(a, b):
    return lax.dot_general(a, b, (((1,), (0,)), ((), ())), preferred_element_type=F32)


def _dot_nt(a, b):
    return lax.dot_general(a, b, (((1,), (1,)), ((), ())), preferred_element_type=F32)


def _pack(val):
    return pltpu.bitcast(val.astype(BF16), U32)


def _unpack(words):
    return pltpu.bitcast(words, BF16)


def _strassen_lhs(a11, a12, a21, a22):
    return a11 + a22, a21 + a22, a11, a22, a11 + a12, a21 - a11, a12 - a22


def _strassen_rhs(b11, b12, b21, b22):
    return b11 + b22, b11, b12 - b22, b21 - b11, b22, b11 + b12, b21 + b22


def _winograd_lhs(a11, a12, a21, a22):
    s1 = a21 + a22
    s2 = s1 - a11
    return a11, a12, a12 - s2, a22, s1, s2, a11 - a21


def _winograd_rhs(b11, b12, b21, b22):
    t1 = b12 - b11
    t2 = b22 - t1
    return b11, b21, b22, b21 - t2, t1, t2, b22 - b12


def _kernel(x_hbm, wq_hbm, wk_hbm, wv_hbm, gw_hbm, wg_hbm, wu_hbm, wd_hbm, wo_hbm, out_ref,
            x_v, wq_v, wg_v, wu_v, wd_v, wo_v,
            wqt_s, qpart_s, lhs_s, lhs2_s, kb_s, qt_s, qf_s, vt_s, g_s,
            wgu_s, wgu_rest_s, wd_s, wd_rest_s, wo_s,
            ot_s, o_s, a_s, gu_s, vbig_s, ring_s, qb_s, b_s, h_s, park_s, stage_s,
            wkv_v, gw_v, sems):
    step = pl.program_id(0)
    tiles = [(s, t) for s in range(NS) for t in range(NT)]
    n = len(tiles)
    on_vpu = [(n - i) * VPU_TILES // n > (n - i - 1) * VPU_TILES // n for i in range(n)]
    slots = [6 if v else 8 for v in on_vpu]
    n_zero = [0]

    def opaque_zero():
        n_zero[0] += 1
        return pl.multiple_of(((step + n_zero[0]) >> 16) * 32, 32)

    def staged_pack(stage, val):
        rows = pl.ds(0, val.shape[0] // 2)
        stage[rows, :] = _pack(val)
        return stage[rows, :]

    def spread_q(block, s, d):
        for c in range(2):
            b11, b21, b12, b22 = [
                jnp.broadcast_to(qf_s[block, pl.ds(DH * (HS * s + c + 2 * u) + HD * v + d, 1), :], (8, TQ))
                for u in range(2) for v in range(2)]
            qb_s[s][:, pl.ds(16 * d + 8 * c, 8), :] = jnp.concatenate(
                _winograd_rhs(b11, b12, b21, b22), axis=0).reshape(7, 8, TQ)

    def vpu_scores(i, stage):
        s, t = tiles[i]
        live = {}

        def product(m, acc):
            rows = pl.ds(opaque_zero(), HD * 16)
            q = qb_s[s][m, rows, :].reshape(HD, 16, TQ)
            k = kb_s[t, m, rows, :]
            q = jnp.concatenate([q[:, :8], q[:, 8:]], axis=2)
            q = jnp.concatenate([q, q], axis=1).reshape(HD * 16, 2 * TQ)
            k = jnp.concatenate([k, k], axis=1)
            for kd, qd in zip(jnp.split(k, HD), jnp.split(q, HD)):
                acc = kd * qd if acc is None else acc + kd * qd
            return acc

        def emit(scores, u, j):
            p = staged_pack(stage, jnp.exp2(scores))
            lhs_s[pl.ds(L_P + 64 * i + 32 * u + 8 * j, 16), :] = jnp.concatenate([p[:, :TQ], p[:, TQ:]], axis=0)

        def c11():
            live["m1"] = product(0, None)
            emit(product(1, live["m1"]), 0, 0)

        def c12():
            live["u2"] = product(5, live.pop("m1"))
            live["m5"] = product(4, None)
            emit(product(2, live["u2"] + live["m5"]), 0, 2)

        def c22():
            live["u3"] = product(6, live.pop("u2"))
            emit(live["u3"] + live.pop("m5"), 1, 2)

        def c21():
            emit(product(3, live.pop("u3")), 1, 0)

        return [(162, c11), (246, c12), (90, c22), (86, c21)]

    @pl.when(step == 0)
    def _load_and_project():
        first, rest = pl.ds(0, X_FIRST), pl.ds(X_FIRST, S - X_FIRST)
        wq, wk, wv, gw, x0, x1, wg, wu, wd, wo = [
            pltpu.make_async_copy(src, dst, sems.at[i]) for i, (src, dst) in enumerate((
                (wq_hbm, wq_v), (wk_hbm, wkv_v.at[0]), (wv_hbm, wkv_v.at[1]), (gw_hbm, gw_v),
                (x_hbm.at[first, :], x_v.at[first, :]), (x_hbm.at[rest, :], x_v.at[rest, :]),
                (wg_hbm, wg_v), (wu_hbm, wu_v), (wd_hbm, wd_v), (wo_hbm, wo_v)))]
        for copy in (wq, wk, wv, gw, x0, x1):
            copy.start()
        lhs_s[pl.ds(L_ZERO, 8), :] = jnp.zeros((8, 128), U32)
        for copy in (wq, wk, wv, gw):
            copy.wait()
        wkv = jnp.concatenate(
            [wkv_v[0].astype(F32), jnp.broadcast_to(gw_v[...].astype(F32).reshape(1, D), (8, D)),
             wkv_v[1].astype(F32)], axis=0).astype(BF16)
        wqt_s[pl.ds(0, D // 2), :] = pltpu.bitcast(wq_v[...].T, U32)
        lane = lax.broadcasted_iota(jnp.int32, (64, 128), 1)
        row = lax.broadcasted_iota(jnp.int32, (24, 128), 0)
        v_big = [jnp.zeros((8, 128), F32)]

        def project_kv(t0):
            kv = _dot_nt(wkv, x_v[pl.ds(128 * t0, 512), :])
            for t in range(t0, t0 + 4):
                kvt = kv[:, 128 * (t - t0):128 * (t - t0 + 1)]
                v_odd = jnp.where(row < 4, 1.0, kvt[24:48])
                vt_s[t, pl.ds(24, 24), :] = v_odd
                vt_s[t, pl.ds(0, 24), :] = jnp.concatenate([v_odd[4:24], jnp.ones((4, 128), F32)], axis=0)
                for r in range(3):
                    v_big[0] = jnp.where(jnp.abs(v_odd[8 * r:8 * r + 8]) <= V_MAX, v_big[0], 1.0)
                k = jnp.concatenate([kvt[0:DH]] * HS + [jnp.zeros((120 - HS * DH, 128), F32),
                                                        jax.nn.sigmoid(kvt[16:24])], axis=0).T
                g_s[pl.ds(128 * t, 128), :] = jnp.broadcast_to(k[:, 124:125], (128, 128))
                words = jnp.where(lane < HS * DH, _pack(k), jnp.zeros((64, 128), U32))
                lhs_s[pl.ds(L_K + 64 * t, 64), :] = words
                lhs2_s[pl.ds(L_K + 64 * t, 64), :] = words
                for d in range(HD):
                    lo = jnp.broadcast_to(k[96:, d:d + 1], (32, 128))
                    hi = jnp.broadcast_to(k[96:, HD + d:HD + d + 1], (32, 128))
                    kb_s[t, :, pl.ds(16 * d, 16), :] = jnp.concatenate(
                        _winograd_lhs(lo[:16], hi[:16], lo[16:], hi[16:]), axis=0).reshape(7, 16, 128)

        def x_terms(t0, t1):
            for t in range(t0, t1):
                for r in range(0, 64, 16):
                    blocks = [x_v[pl.ds(128 * t + 64 * u + r, 16), pl.ds(256 * v, 256)].astype(F32)
                              for u in range(2) for v in range(2)]
                    terms = staged_pack(stage_s[1], jnp.concatenate(_strassen_lhs(*blocks), axis=0))
                    for m, val in enumerate(jnp.split(terms, 7)):
                        for u, dst in enumerate((lhs_s, lhs2_s)):
                            dst[pl.ds(L_X + 512 * t + 64 * m + 32 * u + r // 2, 8), :] = (
                                val[:, 128 * u:128 * (u + 1)])
                    lhs_s[pl.ds(L_X + 512 * t + 448 + r, 16), :] = pltpu.bitcast(
                        x_v[pl.ds(128 * t + 2 * r, 32), pl.ds(512, 128)], U32)

        def gate_up_terms(which, c, r):
            w = (wg_v, wu_v)[which]
            blocks = [w[pl.ds(256 * u + r, 16), pl.ds(128 * (c + 6 * v), 256)].astype(F32)
                      for u in range(2) for v in range(2)]
            terms = staged_pack(stage_s[1], jnp.concatenate(_strassen_rhs(*blocks), axis=0)).reshape(7, 8, 256)
            for u in range(2):
                wgu_s[c + u, :, pl.ds(r // 2, 8), pl.ds(128 * which, 128)] = terms[:, :, 128 * u:128 * (u + 1)]
            if r < 128:
                for v in range(2):
                    val = staged_pack(stage_s[1], w[pl.ds(512 + r, 16), pl.ds(128 * (c + 6 * v), 256)].astype(F32))
                    for u in range(2):
                        wgu_rest_s[c + u, pl.ds(r // 2, 8), pl.ds(256 * v + 128 * which, 128)] = (
                            val[:, 128 * u:128 * (u + 1)])
            wqt_s[pl.ds(D // 2, 8), pl.ds(0, 128)] = wgu_s[c, 0, pl.ds(opaque_zero(), 8), pl.ds(0, 128)]

        def project_q(t0, work=()):
            def lhs(c0, nc, part):
                per = len(work) / (4 * D // 16)
                view = wqt_s.at[pl.ds(opaque_zero(), D // 2)]
                if part is None or not work:
                    return _unpack(view[:, pl.ds(c0, nc)])
                rows = []
                for r in range(D // 16):
                    at = part * D // 16 + r
                    for item in work[int(at * per):int((at + 1) * per)]:
                        item()
                    rows.append(view[pl.ds(8 * r, 8), pl.ds(c0, nc)])
                return _unpack(jnp.concatenate(rows, axis=0))

            q_rest = _dot_nt(lhs(512, 128, None), x_v[pl.ds(128 * t0, 512), pl.ds(512, 128)])
            for u in range(4):
                qpart_s[u] = q_rest[:, 128 * u:128 * (u + 1)]
            for u in range(4):
                q = qpart_s[u, pl.ds(opaque_zero(), D), :] + _dot_nt(
                    lhs(0, 512, u), x_v[pl.ds(128 * (t0 + u), 128), pl.ds(0, 512)])
                q = q * Q_SCALE
                qf_s[t0 + u] = q
                qt_s[t0 + u] = staged_pack(stage_s[1], jnp.concatenate([q, q], axis=1))[:, :128]

        x0.wait()
        wg.start()
        wu.start()
        project_kv(0)
        x_terms(0, 4)
        project_q(0)
        for d in range(HD):
            spread_q(0, 0, d)
        x1.wait()
        wd.start()
        wo.start()
        for t0 in (4, 8, 12):
            project_kv(t0)
        x_terms(4, NQ)
        project_q(4)
        for i in range(AHEAD):
            if on_vpu[i]:
                for _, piece in vpu_scores(i, stage_s[2]):
                    piece()
        project_q(8)
        vbig_s[pl.ds(0, 8), :] = v_big[0]
        wg.wait()
        wu.wait()
        project_q(12, [functools.partial(gate_up_terms, which, c, r)
                       for c in range(0, 6, 2) for r in range(0, 256, 16) for which in range(2)])
        wd.wait()
        for r in range(0, F // 2, 16):
            blocks = [wd_v[pl.ds(F // 2 * u + r, 16), pl.ds(256 * v, 256)].astype(F32)
                      for u in range(2) for v in range(2)]
            wd_s[:, pl.ds(r // 2, 8), :] = staged_pack(
                stage_s[1], jnp.concatenate(_strassen_rhs(*blocks), axis=0)).reshape(7, 8, 256)
        wd_rest_s[...] = pltpu.bitcast(wd_v[:, pl.ds(512, 128)], U32)
        wo.wait()
        for c in range(D // 128):
            wo_s[:, pl.ds(128 * c, 128)] = pltpu.bitcast(wo_v[:, pl.ds(128 * c, 128)], U32)

    zero = opaque_zero()
    next_block = jnp.minimum(step + 1, NQ - 1)

    def queued_spread(block, s, d):
        spread_q(block + opaque_zero(), s, d)
        lhs_s[pl.ds(L_SINK, 8), :] = pltpu.bitcast(qb_s[s][0, pl.ds(opaque_zero(), 8), :], U32)

    queue = []
    for i, (s, t) in enumerate(tiles):
        if on_vpu[i] and i >= AHEAD:
            queue += [(cost, i, piece) for cost, piece in vpu_scores(i, stage_s[0])]
        for d in range(HD):
            if t == (d if s else max(d, AHEAD)):
                where = (step, s + 1) if s + 1 < NS else (next_block, 0)
                queue.append((C_SPREAD, n, functools.partial(queued_spread, *where, d)))
    for i in range(AHEAD):
        if on_vpu[i]:
            queue += [(cost, n, piece) for cost, piece in vpu_scores(i, stage_s[0])]
    capacity = ((300 + 8 * (O_INSIDE + TAIL_SLOTS)) * W_DENSE
                + sum(slots) * W_QK + (n - LAG) * W_PV)
    rate = sum(item[0] for item in queue) / capacity
    credit = [0.0]

    def run_next():
        cost, _, thunk = queue.pop(0)
        credit[0] -= cost
        thunk()

    def paced(load, count, weight):
        rows = []
        for r in range(count):
            credit[0] += weight * rate
            ran = False
            while queue and credit[0] >= queue[0][0] - 1e-6:
                run_next()
                ran = True
            rows.append(load(r, ran))
        return jnp.concatenate(rows, axis=0)

    zeros8 = jnp.zeros((8, TQ), U32)
    sublane = lax.broadcasted_iota(jnp.int32, (8, TQ), 0)
    q_tile, acc, sums = {}, {}, {}

    def q_weights(s):
        base = 40 * s if isinstance(s, int) else pl.multiple_of(40 * s, 8)
        cols = []
        for j in range(HS):
            parts = []
            for r in range(8):
                lo, hi = 10 * j - 8 * r, 10 * j + 10 - 8 * r
                if hi <= 0 or lo >= 8:
                    parts.append(zeros8)
                else:
                    keep = (sublane >= lo) if lo > 0 else (sublane < hi)
                    parts.append(jnp.where(keep, qt_s[step, pl.ds(base + 8 * r, 8), :], zeros8))
            cols.append(jnp.concatenate(parts, axis=0))
        return _unpack(jnp.concatenate(cols, axis=1))

    def scores(i):
        s, t = tiles[i]
        if t == 0:
            q_tile[s] = q_weights(s)
        ordered = lhs_s.at[pl.ds(zero + L_K + 64 * t, 64)]
        free = lhs2_s.at[pl.ds(opaque_zero() + L_K + 64 * t, 64)]
        keys = paced(lambda r, ran: (ordered if ran else free)[pl.ds(8 * r, 8), :], slots[i], W_QK)
        ring_s[i % RING][pl.ds(0, 8 * slots[i]), :] = _pack(jnp.exp2(_dot(_unpack(keys), q_tile[s])))

    def weigh_values(i):
        s, t = tiles[i]
        while any(item[1] <= i for item in queue):
            run_next()
        credit[0] += W_PV * rate
        from_mxu = jnp.split(ring_s[i % RING][pl.ds(zero, 8 * slots[i]), :], HS, axis=1)
        from_vpu = jnp.split(lhs_s[pl.ds(L_P + 64 * i, 64), :], 2 * HS) if on_vpu[i] else []
        values = jnp.split(vt_s[t], 2)
        for j in range(HS):
            r = _dot(values[j % 2], _unpack(jnp.concatenate([from_mxu[j]] + from_vpu[j::HS], axis=0)))
            acc[s, j] = r if t == 0 else r + acc[s, j]

    def normalize(s):
        for j in range(0, HS, 2):
            even, odd = acc.pop((s, j)), acc.pop((s, j + 1))
            total = jnp.where(sublane < 4, odd[0:8], even[16:24])
            sums["min"] = jnp.minimum(sums["min"], total) if sums else total
            sums["all"] = sums["all"] + total if "all" in sums else total
            inv = 1.0 / total
            even = even * jnp.broadcast_to(inv[4:5], (24, TQ))
            odd = odd * jnp.broadcast_to(inv[0:1], (24, TQ))
            ot_s[pl.ds((s * HS + j) * DH, 2 * DH), :] = jnp.concatenate(
                [even[0:16], jnp.where(sublane < 4, even[16:24], odd[0:8]), odd[8:24]], axis=0)

    x_ordered = lhs_s.at[pl.ds(pl.multiple_of(L_X + step * 512, 32), 512)]
    zero_words = lhs_s.at[pl.ds(zero + L_ZERO, 8)]

    def x_rows(bases, count):
        free = lhs2_s.at[pl.ds(pl.multiple_of(L_X + step * 512 + opaque_zero(), 32), 512)]
        return _unpack(paced(lambda r, ran: jnp.concatenate(
            [src[pl.ds(base + 8 * r, 8), :] for src, base in zip((x_ordered, free), bases)], axis=1),
            count, W_DENSE))

    def activation_rows(refs, c0, nc):
        rows = []
        for ref in refs:
            view = ref.at[pl.ds(opaque_zero(), ref.shape[0])]

            def load(r, ran, view=view):
                blk = view[pl.ds(16 * r, 16), pl.ds(c0, nc)]
                if ran:
                    head = blk[0:8, 0:128] + pltpu.bitcast(zero_words[...], F32)
                    blk = jnp.concatenate([jnp.concatenate([head, blk[0:8, 128:]], axis=1), blk[8:]], axis=0)
                return blk

            rows.append(paced(load, ref.shape[0] // 16, W_DENSE))
        return jnp.concatenate(rows, axis=0)

    def park(slot, val):
        park_s[slot][...] = val
        return lambda: park_s[slot][pl.ds(opaque_zero(), 64), :]

    def reglu(gate_up):
        return jnp.maximum(gate_up[:, :128], 0.0) * gate_up[:, 128:]

    def gate_up(c):
        gu_s[...] = _dot(x_rows([448], 8), _unpack(wgu_rest_s[c]))

        def rest(u, v):
            return gu_s[pl.ds(opaque_zero() + 64 * u, 64), pl.ds(256 * v, 256)]

        def product(m):
            return _dot(x_rows([64 * m, 64 * m + 32], 4), _unpack(wgu_s[c, m]))

        m1 = product(0)
        c11 = park(0, m1 + product(6))
        c22 = park(1, m1 + product(5))
        m4 = product(3)
        c11 = park(0, c11() + m4)
        c21 = rest(1, 0) + m4
        m2 = product(1)
        h21 = reglu(c21 + m2)
        c22 = park(1, c22() - m2)
        m5 = product(4)
        h11 = reglu(c11() - m5 + rest(0, 0))
        c12 = rest(0, 1) + m5
        m3 = product(2)
        h12 = reglu(c12 + m3)
        h22 = reglu(c22() + m3 + rest(1, 1))
        for ref, val in zip(h_s, _strassen_lhs(h11, h12, h21, h22) + (h12, h21)):
            ref[:, pl.ds(128 * c, 128)] = val

    def down():
        def product(m):
            r = None
            for u in range(3):
                term = _dot(activation_rows([h_s[m]], 256 * u, 256), _unpack(wd_s[m, pl.ds(128 * u, 128), :]))
                r = term if r is None else term + r
            return r

        m1 = park(0, product(0))
        m6 = product(5)
        c22 = park(1, m1() + m6)
        m7 = product(6)
        c11 = park(0, m1() + m7)
        m4 = product(3)
        c11 = park(0, c11() + m4)
        c21 = park(2, m4)
        m2 = product(1)
        b_s[0][pl.ds(64, 64), pl.ds(0, 256)] = c21() + m2
        c22 = park(1, c22() - m2)
        m5 = product(4)
        b_s[0][pl.ds(0, 64), pl.ds(0, 256)] = c11() - m5
        c12 = park(2, m5)
        m3 = product(2)
        b_s[0][pl.ds(0, 64), pl.ds(256, 256)] = c12() + m3
        b_s[0][pl.ds(64, 64), pl.ds(256, 256)] = c22() + m3

    def down_rest(u):
        left = activation_rows([h_s[2], h_s[8]], 256 * u, 256)
        right = jnp.concatenate([h_s[m][pl.ds(opaque_zero(), 64), pl.ds(256 * u, 256)] for m in (7, 3)], axis=0)
        w = jnp.concatenate([wd_rest_s[pl.ds(384 * v + 128 * u, 128), :] for v in range(2)], axis=0)
        r = _dot(jnp.concatenate([left, right], axis=1), _unpack(w))
        b_s[1][...] = r if u == 0 else b_s[1][pl.ds(opaque_zero(), TQ), :] + r

    def wo_tile(r0, nr, c0, nc):
        return _unpack(wo_s[pl.ds(r0 // 2, nr // 2), pl.ds(c0, nc)])

    def out_proj(c):
        a_s[:, pl.ds(128 * c, 128)] = _dot(activation_rows([o_s], 0, 512), wo_tile(0, 512, 128 * c, 128))

    def mix(a, which):
        g = jnp.concatenate([g_s[pl.ds(pl.multiple_of(step * TQ, TQ), TQ), :]] * (a.shape[1] // 128), axis=1)
        b = b_s[which][pl.ds(opaque_zero(), TQ), :]
        out_ref[:, pl.ds(512 * which, a.shape[1])] = (g * a + (1.0 - g) * b).astype(out_ref.dtype)

    for c in range(6):
        gate_up(c)
    rest_jobs = [functools.partial(down_rest, u) for u in range(3)]
    out_jobs = [functools.partial(out_proj, c) for c in range(O_INSIDE, D // 128)]
    tail = out_jobs + rest_jobs if O_FIRST else rest_jobs + out_jobs
    o_tile_done = {2: 0, 4: 1, 5: 2, 7: 3}
    for i in range(n + LAG):
        if i == DOWN_AT:
            down()
        if i < n:
            scores(i)
        else:
            tail.pop(0)()
        if i >= LAG:
            s, t = tiles[i - LAG]
            weigh_values(i - LAG)
            if t == 2 and s > 0:
                normalize(s - 1)
                if s in o_tile_done:
                    k = 128 * o_tile_done[s]
                    o_s[:, pl.ds(k, 128)] = ot_s[pl.ds(opaque_zero() + k, 128), :].T
            if s == NS - 1 and t in range(4, 4 + 2 * O_INSIDE, 2):
                out_proj((t - 4) // 2)
    normalize(NS - 1)
    for job in tail:
        job()
    while queue:
        run_next()
    o_last = ot_s[pl.ds(opaque_zero() + 512, 128), :].T
    mix(a_s[pl.ds(opaque_zero(), TQ), pl.ds(0, 512)] + _dot(o_last, wo_tile(512, 128, 0, 512)), 0)
    w_last = wo_tile(512, 128, 512, 128)
    mix(a_s[pl.ds(opaque_zero(), TQ), pl.ds(512, 128)]
        + jnp.concatenate([_dot(o_last[32 * r:32 * r + 32], w_last) for r in range(4)], axis=0), 1)

    safe = (sums["min"] >= SUM_MIN) & (sums["all"] <= SUM_MAX) & (vbig_s[pl.ds(0, 8), :] == 0.0)

    @pl.when(jnp.max(jnp.where(safe, 0.0, 1.0)) > 0.0)
    def _redo_with_true_max():
        def slab(s, carry):
            w = q_weights(s)

            def tile_scores(t):
                return _dot(_unpack(lhs_s[pl.ds(opaque_zero() + L_K + 128 * t, 128), :]), w)

            row_max = functools.reduce(jnp.maximum, [
                jnp.max(tile_scores(t).reshape(32, 8, HS * TQ), axis=0) for t in range(NT // 2)])
            row_max = jnp.max(row_max, axis=0, keepdims=True)
            p, o = {}, 0.0
            for t in range(NT // 2 + 2):
                if t < NT // 2:
                    p[t] = jnp.exp2(tile_scores(t) - row_max).astype(BF16)
                if t >= 2:
                    v = jnp.concatenate([vt_s[2 * (t - 2) + u, pl.ds(0, 24), :] for u in range(2)], axis=1)
                    o = o + _dot(v, p.pop(t - 2))
            o = o * (1.0 / o[DH:DH + 1])
            ot_s[pl.ds(pl.multiple_of(s * HS * DH, 8), HS * DH), :] = jnp.concatenate(
                [o[:DH, j * TQ:(j + 1) * TQ] for j in range(HS)], axis=0)
            return carry

        lax.fori_loop(0, NS, slab, 0)
        a = _dot(ot_s[...].T, wo_tile(0, D, 0, D))
        mix(a[:, :512], 0)
        mix(a[:, 512:], 1)


@jax.jit
def pallas_gated_mix__grouped_kv_mqa__glu_gated_reglu__prompt_kernel(
    A_x: jax.Array,
    A_wq: jax.Array,
    A_wk: jax.Array,
    A_wv: jax.Array,
    A_wo: jax.Array,
    B_x: jax.Array,
    B_W_gate: jax.Array,
    B_W_up: jax.Array,
    B_W_down: jax.Array,
    gate_w: jax.Array,
):
    del B_x
    vmem = pltpu.VMEM
    scratch = [
        vmem((S, D), BF16), vmem((D, D), BF16), vmem((D, F), BF16), vmem((D, F), BF16),
        vmem((F, D), BF16), vmem((D, D), BF16),
        vmem((D // 2 + 32, D), U32),
        vmem((4, D, 128), F32),
        vmem((L_ROWS, 128), U32),
        vmem((L_ZERO, 128), U32),
        vmem((NT, 7, HD * 16, 128), F32),
        vmem((NQ, D // 2, TQ), U32),
        vmem((NQ, D, TQ), F32),
        vmem((NT, 48, 128), F32),
        vmem((S, 128), F32),
        vmem((6, 7, 128, 256), U32),
        vmem((6, 64, 512), U32),
        vmem((7, F // 4, 256), U32),
        vmem((F // 2, 128), U32),
        vmem((D // 2, D), U32),
        vmem((D, TQ), F32),
        vmem((TQ, 512), F32),
        vmem((TQ, D), F32),
        vmem((TQ, 512), F32),
        vmem((32, 128), F32),
        [vmem((64, HS * TQ), U32)] * RING,
        [vmem((7, HD * 16, TQ), F32)] * NS,
        [vmem((TQ, 512), F32), vmem((TQ, 128), F32)],
        [vmem((64, F // 2), F32)] * 9,
        [vmem((64, 256), F32)] * 3,
        [vmem((D // 2, 256), U32)] * 3,
        vmem((2, DH, D), BF16),
        vmem((D,), BF16),
        pltpu.SemaphoreType.DMA((10,)),
    ]
    out = pl.pallas_call(
        _kernel,
        grid=(NQ,),
        in_specs=[pl.BlockSpec(memory_space=pl.ANY)] * 9,
        out_specs=pl.BlockSpec((TQ, D), lambda i: (i, 0)),
        out_shape=jax.ShapeDtypeStruct((S, D), A_x.dtype),
        scratch_shapes=scratch,
        compiler_params=pltpu.CompilerParams(
            dimension_semantics=("arbitrary",), vmem_limit_bytes=100 * 2 ** 20),
    )(A_x.reshape(S, D), A_wq, A_wk.T, A_wv.T, gate_w, B_W_gate, B_W_up, B_W_down, A_wo)
    return out.reshape(1, S, D)
```
